```python
import os as _os
_os.environ.setdefault("JAX_PLATFORMS", "cpu")
import jax
import jax.numpy as jnp

def _softmax(x, axis=-1):
    return jax.nn.softmax(x, axis=axis)
def _gelu(x):
    return jax.nn.gelu(x, approximate=True)
def _silu(x):
    return jax.nn.silu(x)
def _sigmoid(x):
    return jax.nn.sigmoid(x)
def _layernorm(x, axis=-1, eps=1e-5):
    m = jnp.mean(x, axis=axis, keepdims=True)
    v = jnp.var(x, axis=axis, keepdims=True)
    return (x - m) / jnp.sqrt(v + eps)
def _scatter_add(tgt, idx, src, axis=0):
    return tgt.at[idx].add(src)
def _segment_sum(src, seg, n):
    return jax.ops.segment_sum(src, seg, n)
class _Rng:
    def __init__(self, key):
        self._k = key
    def _next(self):
        self._k, sub = jax.random.split(self._k)
        return sub
    def normal(self, shape):
        return jax.random.normal(self._next(), shape, dtype=jnp.bfloat16)
    def randint(self, lo, hi, shape):
        return jax.random.randint(self._next(), shape, lo, hi, dtype=jnp.int32)
    def uniform(self, shape, lo=0.0, hi=1.0):
        return jax.random.uniform(self._next(), shape, jnp.bfloat16, lo, hi)
    def permutation(self, n):
        return jax.random.permutation(self._next(), n)


kernel_name = 'interleave_layers__sliding_local_dilated__mixer_channel_mlp__prompt'

def setup_inputs():
    _rng = _Rng(jax.random.key(int.from_bytes(__import__("os").urandom(4), "little")))
    _w = (lambda a: (lambda t: t.astype(jnp.bfloat16) if jnp.issubdtype(t.dtype, jnp.floating) else t)(jnp.asarray(a)))
    def _A_setup():
        B, S, D = 1, 2048, 512
        return {
            "x": _w((lambda *s: _rng.normal(s) * 0.05)(B, S, D)),
            "wqkv": _w((lambda *s: _rng.normal(s) * 0.05)(D, 3 * D)),
            "wo": _w((lambda *s: _rng.normal(s) * 0.05)(D, D)),
        }
    _A_in = _A_setup()

    def _B_setup():
        B, S, D, F = 1, 2048, 512, 1376
        return {
            "x": _w((lambda *s: _rng.normal(s) * 0.05)(B, S, D)),
            "w1": _w((lambda *s: _rng.normal(s) * 0.4)(D, F) * (D ** -0.5)),
            "b1": _w((lambda *s: _rng.normal(s) * 0.4)(F)),
            "w2": _w((lambda *s: _rng.normal(s) * 0.4)(F, D) * (F ** -0.5)),
            "b2": _w((lambda *s: _rng.normal(s) * 0.4)(D)),
        }
    _B_in = _B_setup()

    return {
        "A_x": _A_in["x"],
        "A_wqkv": _A_in["wqkv"],
        "A_wo": _A_in["wo"],
        "B_x": _B_in["x"],
        "B_w1": _B_in["w1"],
        "B_b1": _B_in["b1"],
        "B_w2": _B_in["w2"],
        "B_b2": _B_in["b2"],
    }

def reference(A_x, A_wqkv, A_wo, B_x, B_w1, B_b1, B_w2, B_b2):
    def _A_ref(x, wqkv, wo):
        B, S, D = x.shape
        H = 32; Dh = D // H
        W, dil = 8, 2
        qkv = (lambda x, *d: x.transpose(*d))((x @ wqkv).reshape(B, S, 3, H, Dh), 2, 0, 3, 1, 4)
        q, k, v = qkv[0], qkv[1], qkv[2]
        scale = Dh ** -0.5
        pos = jnp.arange(S)
        off = jnp.arange(W) * dil
        idx = pos[:, None] - off[None, :]
        mask = idx >= 0
        idx_c = jnp.where(mask, idx, 0).reshape(-1)
        kg = k[:, :, idx_c, :].reshape(B, H, S, W, Dh)
        vg = v[:, :, idx_c, :].reshape(B, H, S, W, Dh)
        logits = jnp.einsum("bhsd,bhswd->bhsw", q, kg) * scale
        logits = jnp.where(mask[None, None, :, :], logits, -1e9)
        attn = _softmax(logits, axis=-1)
        o = jnp.einsum("bhsw,bhswd->bhsd", attn, vg)
        return (lambda x, *d: x.transpose(*d))(o, 0, 2, 1, 3).reshape(B, S, D) @ wo

    def _B_ref(x, w1, b1, w2, b2):
        y = _layernorm(x, axis=-1)
        h = _gelu(jnp.einsum("bsd,df->bsf", y, w1) + b1)
        return jnp.einsum("bsf,fd->bsd", h, w2) + b2

    x = A_x
    x = x + _A_ref(_layernorm(x, axis=-1), A_wqkv, A_wo)
    x = x + _B_ref(_layernorm(x, axis=-1), B_w1, B_b1, B_w2, B_b2)
    x = x + _A_ref(_layernorm(x, axis=-1), A_wqkv, A_wo)
    x = x + _B_ref(_layernorm(x, axis=-1), B_w1, B_b1, B_w2, B_b2)
    return x
```

```python
import functools, math
import jax
import jax.numpy as jnp
from jax import lax
import jax.experimental.pallas as pl
import jax.experimental.pallas.tpu as pltpu

S, D, F = 2048, 512, 1376
FP = 1408
H, DH, W, DIL = 32, 16, 8, 2
HALO = 16
EPS = 1e-5
LOG2E = 1.4426950408889634
QSCALE = (DH ** -0.5) * LOG2E
NEG = -1e9 * LOG2E
f32, bf16, u32 = jnp.float32, jnp.bfloat16, jnp.uint32


def _ln(x):
    m = jnp.mean(x, axis=-1, keepdims=True)
    xc = x - m
    v = jnp.mean(xc * xc, axis=-1, keepdims=True)
    return xc * lax.rsqrt(v + EPS)


def _gelu(x):
    c = math.sqrt(2.0 / math.pi)
    inner = x * (c + (c * 0.044715) * (x * x))
    return (0.5 * x) * (1.0 + jnp.tanh(inner))


def _wload(ref, k0, k1, n0, n1):
    return pltpu.bitcast(ref[k0 // 2:k1 // 2, n0:n1], bf16)


def _dot(a, b):
    return jnp.dot(a, b, preferred_element_type=f32)


def _dot_t(a, b):
    return lax.dot_general(a, b, (((1,), (1,)), ((), ())), preferred_element_type=f32)


def make_kernel(M, RC):
    NB = S // M

    def kernel(x_hbm, wqkv_hbm, wo_hbm, w1t_hbm, b1_hbm, w2_hbm, b2_hbm, o_hbm,
               x_v, o_v, wqkv_v, wo_v, w1_v, w2_v, b1_v, b2_v,
               wqkv_p, wo_p, w1_p, w2_p, b1_p, b2_p, wo_tmp, kv, y1_s, xa_s, xb_s, sems, osem):

        cp_x01 = pltpu.make_async_copy(x_hbm.at[0:2 * M], x_v.at[0:2 * M], sems.at[0])
        cp_wqkv = [pltpu.make_async_copy(wqkv_hbm.at[:, t * D:(t + 1) * D], wqkv_v.at[:, t * D:(t + 1) * D],
                                         sems.at[1 + t]) for t in range(3)]
        cp_wo = pltpu.make_async_copy(wo_hbm, wo_v, sems.at[4])
        cp_b1 = pltpu.make_async_copy(b1_hbm, b1_v, sems.at[5])
        cp_b2 = pltpu.make_async_copy(b2_hbm, b2_v, sems.at[6])
        cp_w1 = pltpu.make_async_copy(w1t_hbm, w1_v.at[0:F], sems.at[7])
        cp_w2 = pltpu.make_async_copy(w2_hbm, w2_v.at[0:F], sems.at[8])
        cp_xr = pltpu.make_async_copy(x_hbm.at[2 * M:S], x_v.at[2 * M:S], sems.at[9])

        def out_copy(n):
            r = n * M
            if not isinstance(n, int):
                r = pl.multiple_of(r, M)
            return pltpu.make_async_copy(o_v.at[pl.ds(r, M)], o_hbm.at[pl.ds(r, M)], osem)

        for cp in [cp_x01, cp_wqkv[0], cp_wqkv[1], cp_wqkv[2], cp_wo, cp_b1, cp_b2, cp_w1, cp_w2, cp_xr]:
            cp.start()

        lane = lax.broadcasted_iota(jnp.int32, (8, 128), 1)
        dq = (lane % 16) // 4
        g_, j_, h_ = lane // 32, (lane % 32) // 8, lane % 8
        idx = [h_ * 16 + 4 * ((i + j_) % 4) + g_ for i in range(4)]
        msk = [dq == t for t in range(4)]

        def perm_qkv(t):
            for r in range(D // 16):
                src = [pltpu.bitcast(wqkv_v[r * 16:(r + 1) * 16, t * D + j * 128: t * D + (j + 1) * 128], u32)
                       for j in range(4)]
                for i in range(4):
                    m = src[(0 - i) % 4]
                    for tq in range(1, 4):
                        m = jnp.where(msk[tq], src[(tq - i) % 4], m)
                    wqkv_p[r * 8:(r + 1) * 8, t * D + i * 128: t * D + (i + 1) * 128] = \
                        jnp.take_along_axis(m, idx[i], axis=1)

        def perm_wo():
            for cb in range(4):
                wo_tmp[cb] = wo_v[:, cb * 128:(cb + 1) * 128].astype(f32)
            for cb in range(4):
                for i in range(4):
                    for g in range(4):
                        rows = [wo_tmp[cb, pl.ds(j * 128 + 4 * ((i + j) % 4) + g, 8, stride=16), :] for j in range(4)]
                        blk = jnp.concatenate(rows, axis=0).astype(bf16)
                        r0 = (i * 128 + g * 32) // 2
                        wo_p[r0:r0 + 16, cb * 128:(cb + 1) * 128] = pltpu.bitcast(blk, u32)

        def rows_map(fn, x):
            return jnp.concatenate([fn(x[r:r + RC]) for r in range(0, x.shape[0], RC)], axis=0)

        def ln1(x):
            return rows_map(_ln, x).astype(bf16)

        def ln2(x):
            return rows_map(lambda a: _ln(_ln(a)), x).astype(bf16)

        def q_tile(y, layer, c, row0=HALO):
            r = _dot(y, _wload(wqkv_p, 0, D, c * 128, (c + 1) * 128))
            if c < 4:
                return r * QSCALE
            kv[layer * 8 + c - 4, row0:row0 + y.shape[0], :] = r
            return None

        def mm_Q(y, layer):
            qs = [q_tile(y, layer, c) for c in range(12)]
            return qs[:4]

        def halo(layer, end):
            L = layer * 8
            kv[L:L + 8, 0:HALO, :] = kv[L:L + 8, end - HALO:end, :]

        def attn(q, layer, first, row0=HALO):
            L = layer * 8
            outs = []
            for r0 in range(0, M, RC):
                g0 = row0 + r0
                qs = [q[j][r0:r0 + RC] for j in range(4)]
                ls = []
                for w in range(W):
                    s = None
                    for j in range(4):
                        t_ = qs[j] * kv[L + j, pl.ds(g0 - DIL * w, RC), :]
                        s = t_ if s is None else s + t_
                    s = s + pltpu.roll(s, 64, 1)
                    s = s + pltpu.roll(s, 32, 1)
                    if first and r0 < HALO and w > 0:
                        row = r0 + lax.broadcasted_iota(jnp.int32, (RC, 128), 0)
                        s = jnp.where(row >= DIL * w, s, NEG)
                    ls.append(s)
                m = ls[0]
                for w in range(1, W):
                    m = jnp.maximum(m, ls[w])
                ps = [jnp.exp2(l - m) for l in ls]
                den = ps[0]
                for w in range(1, W):
                    den = den + ps[w]
                inv = 1.0 / den
                oj = []
                for j in range(4):
                    a = None
                    for w in range(W):
                        t_ = ps[w] * kv[L + 4 + j, pl.ds(g0 - DIL * w, RC), :]
                        a = t_ if a is None else a + t_
                    oj.append(a * inv)
                outs.append(jnp.concatenate(oj, axis=1))
            return jnp.concatenate(outs, axis=0).astype(bf16)

        def mm_W(x, o):
            return x + _dot(o, _wload(wo_p, 0, D, 0, D))

        def mm_M1(y, repack=False):
            hs = []
            for n0 in range(0, FP, 128):
                if repack:
                    w = w1_v[n0:n0 + 128, :]
                    w1_p[n0 // 2:n0 // 2 + 64, :] = pltpu.bitcast(w, u32)
                else:
                    w = _wload(w1_p, n0, n0 + 128, 0, D)
                hs.append(_gelu(_dot_t(y, w) + b1_p[:, n0:n0 + 128]))
            return jnp.concatenate(hs, axis=1).astype(bf16)

        def mm_M2(x, h, repack=False):
            if repack:
                w = w2_v[...]
                w2_p[...] = pltpu.bitcast(w, u32)
            else:
                w = _wload(w2_p, 0, FP, 0, D)
            return x + _dot(h, w) + b2_p[...]

        def xblk(n):
            r = n * M
            if not isinstance(n, int):
                r = pl.multiple_of(r, M)
            return x_v[pl.ds(r, M), :].astype(f32)

        def y1_load():
            return pltpu.bitcast(y1_s[...], bf16)

        def y1_next(n):
            y1_s[...] = pltpu.bitcast(ln1(xblk(n)), u32)

        def put_out(n, val):
            r = n * M
            if not isinstance(n, int):
                r = pl.multiple_of(r, M)
            o_v[pl.ds(r, M), :] = val.astype(bf16)
            out_copy(n).start()

        kv[:, 0:HALO, :] = jnp.zeros((16, HALO, 128), f32)
        w1_v[F:FP, :] = jnp.zeros((FP - F, D), bf16)
        w2_v[F:FP, :] = jnp.zeros((FP - F, D), bf16)
        cp_x01.wait()
        x01 = x_v[0:2 * M, :].astype(f32)
        y01 = ln1(x01)
        q01 = []
        cp_wqkv[0].wait()
        perm_qkv(0)
        q01 += [q_tile(y01, 0, 0), q_tile(y01, 0, 1)]
        cp_wqkv[1].wait()
        perm_qkv(1)
        q01 += [q_tile(y01, 0, 2), q_tile(y01, 0, 3)]
        q_tile(y01, 0, 4); q_tile(y01, 0, 5)
        cp_wqkv[2].wait()
        perm_qkv(2)
        q_tile(y01, 0, 6); q_tile(y01, 0, 7)
        q_tile(y01, 0, 8); q_tile(y01, 0, 9)
        cp_wo.wait()
        cp_b1.wait()
        cp_b2.wait()
        perm_wo()
        b1_p[:, 1280:FP] = jnp.zeros((1, 128), f32)
        b1_p[:, 0:F] = b1_v[...].astype(f32).reshape(1, F)
        b2_p[...] = b2_v[...].astype(f32).reshape(1, D)
        q_tile(y01, 0, 10); q_tile(y01, 0, 11)
        x0 = mm_W(x01[0:M], attn([q[0:M] for q in q01], 0, True))
        x1 = mm_W(x01[M:2 * M], attn([q[M:2 * M] for q in q01], 0, False, row0=HALO + M))
        halo(0, HALO + 2 * M)
        cp_w1.wait()
        h0 = mm_M1(ln2(x0), repack=True)
        h1 = mm_M1(ln2(x1))
        cp_w2.wait()
        x0 = mm_M2(x0, h0, repack=True)
        xa_s[...] = mm_M2(x1, h1)
        q2 = mm_Q(ln1(x0), 1)
        cp_xr.wait()
        y1_next(2)
        xb_s[...] = mm_W(x0, attn(q2, 1, True))
        halo(1, HALO + M)

        def body(n, carry):
            x1 = xa_s[...]
            x2 = xb_s[...]
            q = mm_Q(y1_load(), 0)
            h2 = mm_M1(ln2(x2))
            put_out(n - 2, mm_M2(x2, h2))
            x = mm_W(xblk(n), attn(q, 0, False))
            halo(0, HALO + M)
            q2 = mm_Q(ln1(x1), 1)
            h = mm_M1(ln2(x))
            xa_s[...] = mm_M2(x, h)
            xb_s[...] = mm_W(x1, attn(q2, 1, False))
            halo(1, HALO + M)
            y1_next(jnp.minimum(n + 1, NB - 1))
            return carry
        lax.fori_loop(2, NB, body, 0)

        x1 = xa_s[...]
        x2 = xb_s[...]
        q2 = mm_Q(ln1(x1), 1)
        h2 = mm_M1(ln2(x2))
        put_out(NB - 2, mm_M2(x2, h2))
        x2 = mm_W(x1, attn(q2, 1, False))
        h2 = mm_M1(ln2(x2))
        put_out(NB - 1, mm_M2(x2, h2))
        pltpu.make_async_copy(o_v, o_hbm, osem).wait()

    return kernel


def build(M=128, RC=16):
    NB = S // M

    @jax.jit
    def fn(A_x, A_wqkv, A_wo, B_x, B_w1, B_b1, B_w2, B_b2):
        x = A_x.reshape(S, D)
        anyspec = pl.BlockSpec(memory_space=pl.ANY)
        out = pl.pallas_call(
            make_kernel(M, RC),
            in_specs=[anyspec] * 7,
            out_specs=anyspec,
            out_shape=jax.ShapeDtypeStruct((S, D), bf16),
            scratch_shapes=[
                pltpu.VMEM((S, D), bf16), pltpu.VMEM((S, D), bf16),
                pltpu.VMEM((D, 3 * D), bf16), pltpu.VMEM((D, D), bf16),
                pltpu.VMEM((FP, D), bf16), pltpu.VMEM((FP, D), bf16),
                pltpu.VMEM((F,), bf16), pltpu.VMEM((D,), bf16),
                pltpu.VMEM((D // 2, 3 * D), u32), pltpu.VMEM((D // 2, D), u32),
                pltpu.VMEM((FP // 2, D), u32), pltpu.VMEM((FP // 2, D), u32),
                pltpu.VMEM((1, FP), f32), pltpu.VMEM((1, D), f32), pltpu.VMEM((4, D, 128), f32),
                pltpu.VMEM((16, 2 * M + HALO, 128), f32),
                pltpu.VMEM((M // 2, D), u32), pltpu.VMEM((M, D), f32), pltpu.VMEM((M, D), f32),
                pltpu.SemaphoreType.DMA((10,)), pltpu.SemaphoreType.DMA(()),
            ],
            compiler_params=pltpu.CompilerParams(vmem_limit_bytes=100 << 20),
        )(x, A_wqkv, A_wo, B_w1.T, B_b1, B_w2, B_b2)
        return out.reshape(1, S, D)
    return fn


pallas_interleave_layers__sliding_local_dilated__mixer_channel_mlp__prompt_kernel = build(M=128)
```

```python
import functools, math
import jax
import jax.numpy as jnp
import numpy as np
from jax import lax
import jax.experimental.pallas as pl
import jax.experimental.pallas.tpu as pltpu

S, D, F = 2048, 512, 1376
FP = 1408
H, DH, W, DIL = 32, 16, 8, 2
HALO = 16
WS = 20
EPS = 1e-5
LOG2E = 1.4426950408889634
QSCALE = (DH ** -0.5) * LOG2E
QSCALE_BITS = int(np.float32(QSCALE).view(np.uint32))
NEG = -1e9 * LOG2E
f32, bf16, u32 = jnp.float32, jnp.bfloat16, jnp.uint32


def _ln(x):
    m = jnp.mean(x, axis=-1, keepdims=True)
    xc = x - m
    v = jnp.mean(xc * xc, axis=-1, keepdims=True)
    return xc * lax.rsqrt(v + EPS)


def _gelu(x):
    c = math.sqrt(2.0 / math.pi)
    inner = x * (c + (c * 0.044715) * (x * x))
    return (0.5 * x) * (1.0 + jnp.tanh(inner))


def _dot(a, b):
    return jnp.dot(a, b, preferred_element_type=f32)


def _dot_t(a, b):
    return lax.dot_general(a, b, (((1,), (1,)), ((), ())), preferred_element_type=f32)


class _Scopes:
    def __init__(self, on):
        self.on, self.cur = on, None

    def __call__(self, name):
        if not self.on:
            return
        if self.cur is not None:
            self.cur.__exit__(None, None, None)
            self.cur = None
        if name is not None:
            self.cur = jax.named_scope(name)
            self.cur.__enter__()


def make_kernel(M, RC, RA, scopes, U, NTAIL, nb, dl, lag, nb0, wodl, pa, pb, edl, esplit, gd, gs, gx):
    NB = S // M
    P = 3
    NC = M // RA

    def kernel(x_hbm, wqkv_hbm, wo_hbm, w1t_hbm, b1_hbm, w2_hbm, b2_hbm, o_hbm,
               x_v, o_v, wqkv_v, wo_v, w1_v, w2_v, b1_v, b2_v,
               wqkv_p, wo_p, w1_p, w2_p, b1_p, b2_p, wo_tmp, kv, y2_s, q_s, xa_s, xb_s, zero_s, sems, osem):
        scope = _Scopes(scopes)
        wcount = [0]

        def wait(*cps):
            wcount[0] += 1
            scope("W%d" % wcount[0])
            for cp in cps:
                cp.wait()
            scope("R%d" % wcount[0])

        scope("R0")
        XE = (P + 1) * M
        cp_x0 = pltpu.make_async_copy(x_hbm.at[0:M], x_v.at[0:M], sems.at[0])
        cp_x123 = pltpu.make_async_copy(x_hbm.at[M:XE], x_v.at[M:XE], sems.at[11])
        cp_wq = [pltpu.make_async_copy(wqkv_hbm.at[hf * 256:(hf + 1) * 256, 0:D], wqkv_v.at[hf * 256:(hf + 1) * 256, 0:D],
                                       sems.at[(1, 9)[hf]]) for hf in range(2)]
        cp_wqkv = [None] + [pltpu.make_async_copy(wqkv_hbm.at[:, t * D:(t + 1) * D], wqkv_v.at[:, t * D:(t + 1) * D],
                                                  sems.at[1 + t]) for t in range(1, 3)]
        cp_wo = pltpu.make_async_copy(wo_hbm, wo_v, sems.at[4])
        cp_b1 = pltpu.make_async_copy(b1_hbm, b1_v, sems.at[5])
        cp_b2 = pltpu.make_async_copy(b2_hbm, b2_v, sems.at[6])
        cp_w1 = pltpu.make_async_copy(w1t_hbm, w1_v.at[0:F], sems.at[7])
        cp_w2 = pltpu.make_async_copy(w2_hbm, w2_v.at[0:F], sems.at[8])
        cp_xr = pltpu.make_async_copy(x_hbm.at[XE:S], x_v.at[XE:S], sems.at[10])

        def rowslice(n):
            r = n * M
            if not isinstance(n, int):
                r = pl.multiple_of(r, M)
            return pl.ds(r, M)

        for cp in [cp_x0, cp_wq[0], cp_wq[1], cp_x123, cp_wqkv[1], cp_wqkv[2], cp_wo, cp_b1, cp_b2, cp_w1, cp_w2, cp_xr]:
            cp.start()

        lane = lax.broadcasted_iota(jnp.int32, (8, 128), 1)
        dq = (lane % 16) // 4
        g_, j_, h_ = lane // 32, (lane % 32) // 8, lane % 8
        idx = [h_ * 16 + 4 * ((i + j_) % 4) + g_ for i in range(4)]
        msk = [dq == t for t in range(4)]

        def perm_qkv(t, tiles=(0, 1, 2, 3), rows=range(D // 16)):
            for i in tiles:
                for r in rows:
                    src = [pltpu.bitcast(wqkv_v[r * 16:(r + 1) * 16, t * D + j * 128: t * D + (j + 1) * 128], u32)
                           for j in range(4)]
                    m = src[(0 - i) % 4]
                    for tq in range(1, 4):
                        m = jnp.where(msk[tq], src[(tq - i) % 4], m)
                    wqkv_p[r * 8:(r + 1) * 8, t * D + i * 128: t * D + (i + 1) * 128] = \
                        jnp.take_along_axis(m, idx[i], axis=1)

        def perm_wo_a(cb, j):
            for hh in range(8 * j, 8 * j + 8):
                wo_tmp[cb, hh * WS:hh * WS + DH, :] = wo_v[hh * DH:(hh + 1) * DH, cb * 128:(cb + 1) * 128].astype(f32)

        def perm_wo_b(cb, i):
            for g in range(4):
                rows = [wo_tmp[cb, pl.ds(j * 8 * WS + 4 * ((i + j) % 4) + g, 8, stride=WS), :] for j in range(4)]
                blk = pltpu.bitcast(jnp.concatenate(rows, axis=0).astype(bf16), u32)
                r0 = (i * 128 + g * 32) // 2
                wo_p[r0:r0 + 16, cb * 128:(cb + 1) * 128] = blk

        def perm_wo_pieces():
            return [functools.partial(fn, cb, t) for cb in range(4) for fn in (perm_wo_a, perm_wo_b) for t in range(4)]

        def ztok(pieces):
            bits = [pltpu.bitcast(p, u32) for p in pieces]
            return functools.reduce(lambda u, v: u | v, bits) & zero_s[...]

        def pieces_of(a):
            return [a[r:r + 8, c:c + 128] for r in range(0, a.shape[0], 8) for c in range(0, a.shape[1], 128)]

        def patch(wu, r, tok):
            rows = wu[r:r + 8]
            if wu.shape[1] > 128:
                rows = jnp.concatenate([rows[:, 0:128] | tok, rows[:, 128:]], axis=1)
            else:
                rows = rows | tok
            parts = ([wu[:r]] if r > 0 else []) + [rows] + ([wu[r + 8:]] if r + 8 < wu.shape[0] else [])
            return jnp.concatenate(parts, axis=0)

        class Timeline:
            def __init__(self):
                self.slot, self.due, self.trig = 0, {}, {}

            def deadline(self, slot, fn):
                self.due.setdefault(slot, []).append(fn)

            def trigger(self, slot, fn):
                self.trig.setdefault(slot, []).append(fn)

            def weights(self, wu, r=0, off=0):
                for fn in self.due.pop(self.slot + off, []):
                    wu = patch(wu, r, fn())
                return wu

            def done(self, r, n=1):
                lo = self.slot
                self.slot += n
                for s in range(lo, self.slot):
                    for fn in self.trig.pop(s, []):
                        fn(r[r.shape[0] - 8:, 0:128])
        tl = Timeline()

        def rel(offs):
            return [tl.slot + o for o in offs]

        def rows_map(fn, x):
            return jnp.concatenate([fn(x[r:r + RC]) for r in range(0, x.shape[0], RC)], axis=0)

        def ln1(x):
            return rows_map(_ln, x).astype(bf16)

        def ln2(x):
            return rows_map(lambda a: _ln(_ln(a)), x).astype(bf16)

        def halo(layer, end):
            L = layer * 8
            kv[L:L + 8, 0:HALO, :] = kv[L:L + 8, end - HALO:end, :]

        class Attn:
            def __init__(self, layer, first=False, row0=HALO):
                self.layer, self.first, self.row0 = layer, first, row0
                self.q = [None] * 4
                self.half, self.logit, self.outs, self.timed = {}, {}, {}, set()

            def qk(self, c, tok=None):
                L, r0 = self.layer * 8, c * RA
                g0 = self.row0 + r0
                if tok is None:
                    sc_ = QSCALE
                else:
                    sc8 = pltpu.bitcast(tok | QSCALE_BITS, f32)
                    sc_ = jnp.concatenate([sc8] * (RA // 8), axis=0)
                qs = [self.q[j][r0:r0 + RA] * sc_ for j in range(4)]
                ls = []
                for w in range(W):
                    s = None
                    for j in range(4):
                        t_ = qs[j] * kv[L + j, pl.ds(g0 - DIL * w, RA), :]
                        s = t_ if s is None else s + t_
                    ls.append(s)
                self.half[c] = [s + pltpu.roll(s, 64, 1) for s in ls]
                for c2 in sorted(self.half):
                    if c2 <= c - lag:
                        self.qkb(c2)

            def qkb(self, c):
                r0 = c * RA
                ls = [s + pltpu.roll(s, 32, 1) for s in self.half.pop(c)]
                if self.first and r0 < HALO:
                    row = r0 + lax.broadcasted_iota(jnp.int32, (RA, 128), 0)
                    ls = [ls[0]] + [jnp.where(row >= DIL * w, ls[w], NEG) for w in range(1, W)]
                self.logit[c] = ls

            def qk_all(self):
                for c in range(NC):
                    self.qk(c)
                for c in sorted(self.half):
                    self.qkb(c)

            def av(self, c):
                L, r0 = self.layer * 8, c * RA
                g0 = self.row0 + r0
                ls = self.logit[c]
                m = ls[0]
                for w in range(1, W):
                    m = jnp.maximum(m, ls[w])
                ps = [jnp.exp2(l - m) for l in ls]
                den = ps[0]
                for w in range(1, W):
                    den = den + ps[w]
                inv = 1.0 / den
                oj = []
                for j in range(4):
                    a = None
                    for w in range(W):
                        t_ = ps[w] * kv[L + 4 + j, pl.ds(g0 - DIL * w, RA), :]
                        a = t_ if a is None else a + t_
                    oj.append(a * inv)
                self.outs[c] = jnp.concatenate(oj, axis=1)

            def finish(self, c):
                for c2 in range(c, min(c + lag + 1, NC)):
                    if c2 not in self.logit and c2 not in self.half and not (c2 in self.timed and c2 > c):
                        self.qk(c2)
                if c in self.half:
                    self.qkb(c)
                if c not in self.outs:
                    self.av(c)

            def start_at(self, slots):
                for c, s in enumerate(slots):
                    self.timed.add(c)
                    tl.trigger(s, lambda piece, c=c: self.qk(c, ztok([piece])))

            def due_at(self, slots):
                def tok(c):
                    self.finish(c)
                    return ztok(pieces_of(self.outs[c]))
                for c, s in enumerate(slots):
                    tl.deadline(s, lambda c=c: tok(c))

            def done(self):
                for c in range(NC):
                    self.finish(c)
                return jnp.concatenate([self.outs[c] for c in range(NC)], axis=0).astype(bf16)

        def q_tile(y, layer, c, row0=HALO):
            wu = tl.weights(wqkv_p[:, c * 128:(c + 1) * 128])
            r = _dot(y, pltpu.bitcast(wu, bf16))
            if c >= 4:
                kv[layer * 8 + c - 4, row0:row0 + y.shape[0], :] = r
            tl.done(r, y.shape[0] // 128)
            return r

        def mm_Q(y, layer, first=False, nb_=None, dl_=None, row0=HALO):
            at = Attn(layer, first=first, row0=row0)
            end = tl.slot + 12
            if nb_ is not None:
                at.start_at([end + s for s in nb_])
            if dl_ is not None:
                at.due_at([end + s for s in dl_])
            for c in range(12):
                r = q_tile(y, layer, c, row0=row0)
                if c < 4:
                    at.q[c] = r
            return at

        def mm_W(x, o):
            outs = []
            for j in range(4):
                cs = slice(j * 128, (j + 1) * 128)
                wu = tl.weights(wo_p[:, cs])
                r = _dot(o, pltpu.bitcast(wu, bf16))
                tl.done(r)
                outs.append(x[:, cs] + r)
            return jnp.concatenate(outs, axis=1)

        def mm_M1(y, repack=False):
            hs = []
            for t in range(FP // 128):
                n0 = t * 128
                if repack:
                    wu = pltpu.bitcast(w1_v[n0:n0 + 128, :], u32)
                    w1_p[n0 // 2:n0 // 2 + 64, :] = wu
                else:
                    wu = w1_p[n0 // 2:n0 // 2 + 64, :]
                r = _dot_t(y, pltpu.bitcast(tl.weights(wu), bf16))
                tl.done(r)
                hs.append(_gelu(r + b1_p[:, n0:n0 + 128]))
                if gd and t + gd < FP // 128 + gx:
                    tl.deadline(tl.slot - 1 + gd, lambda hh=hs[-1]: ztok(pieces_of(hh)[gs - 1::gs]))
            return jnp.concatenate(hs, axis=1).astype(bf16)

        def mm_M2(x, h, repack=False, js=(0, 1, 2, 3)):
            outs = []
            for j in js:
                cs = slice(j * 128, (j + 1) * 128)
                if repack:
                    wu = pltpu.bitcast(w2_v[:, cs], u32)
                    w2_p[:, cs] = wu
                else:
                    wu = w2_p[:, cs]
                ps = [p for p in range(11) if (4 * p) // 11 == j]
                for i, p in enumerate(ps):
                    wu = tl.weights(wu, ((4 * p) % 11) * 64, off=i)
                r = _dot(h, pltpu.bitcast(wu, bf16))
                tl.done(r, len(ps))
                outs.append(x[:, cs] + r + b2_p[:, cs])
            return jnp.concatenate(outs, axis=1)

        def xblk(n):
            return x_v[rowslice(n), :].astype(f32)

        def put_out(n, val, c0=0):
            cs = slice(c0, c0 + val.shape[1])
            o_v[rowslice(n), cs] = val.astype(bf16)
            pltpu.make_async_copy(o_v.at[rowslice(n), cs], o_hbm.at[rowslice(n), cs], osem).start()

        class State:
            at = None
            x1 = None
            x2 = None
            y2 = None

            def save(self):
                xa_s[...] = self.x1
                xb_s[...] = self.x2
                y2_s[...] = pltpu.bitcast(self.y2, u32)
                q_s[...] = jnp.concatenate(self.at.q, axis=1)
                tl.due.clear()
                tl.trig.clear()

            def load(self):
                self.x1 = xa_s[...]
                self.x2 = xb_s[...]
                self.y2 = pltpu.bitcast(y2_s[...], bf16)
                self.at = Attn(0)
                self.at.q = [q_s[:, j * 128:(j + 1) * 128] for j in range(4)]
                if nb0 is not None:
                    self.at.start_at(rel(nb0))
                self.at.due_at(rel(dl))

        def ln2s(x):
            return ln2(x)

        def step(st, n, last_in_block=False):
            x1, x2, at = st.x1, st.x2, st.at
            h2 = mm_M1(st.y2)
            put_out(n - 2, mm_M2(x2, h2))
            x = mm_W(xblk(n), at.done())
            halo(0, HALO + M)
            at = mm_Q(ln1(x1), 1, nb_=nb, dl_=dl)
            h = mm_M1(ln2(x))
            st.x1 = mm_M2(x, h)
            st.x2 = mm_W(x1, at.done())
            halo(1, HALO + M)
            st.y2 = ln2s(st.x2)
            if not (isinstance(n, int) and n + 1 >= NB):
                if last_in_block:
                    st.at = mm_Q(ln1(xblk(n + 1)), 0)
                else:
                    st.at = mm_Q(ln1(xblk(n + 1)), 0, nb_=nb, dl_=dl)

        PB = 2 * HALO + M
        kv[:, PB - HALO:PB, :] = jnp.zeros((16, HALO, 128), f32)
        zero_s[...] = jnp.zeros((8, 128), u32)
        w1_v[F:FP, :] = jnp.zeros((FP - F, D), bf16)
        w2_v[F:FP, :] = jnp.zeros((FP - F, D), bf16)
        ats = [Attn(0, first=(b == 0), row0=PB + b * M) for b in range(P)] + [Attn(0)]

        def qt(b, cs):
            for c in cs:
                r = q_tile(ys[b], 0, c, row0=ats[b].row0)
                if c < 4:
                    ats[b].q[c] = r

        def wblk(b):
            xs[b] = mm_W(xs[b], ats[b].done())

        def qhalf(hf, c):
            w = pltpu.bitcast(wqkv_p[hf * 128:(hf + 1) * 128, c * 128:(c + 1) * 128], bf16)
            return _dot(ys[0][:, hf * 256:(hf + 1) * 256], w)

        wait(cp_x0)
        xs = [xblk(0)]
        ys = [ln1(xs[0])]
        wait(cp_wq[0])
        perm_qkv(0, rows=range(0, 16))
        for c in range(4):
            q_s[:, c * 128:(c + 1) * 128] = qhalf(0, c)
        wait(cp_wq[1])
        perm_qkv(0, rows=range(16, 32))
        for c in range(pa):
            ats[0].q[c] = q_s[:, c * 128:(c + 1) * 128] + qhalf(1, c)
        wait(cp_x123)
        xs += [xblk(1), xblk(2)]
        ys += [ln1(xs[1]), ln1(xs[2]), ln1(xblk(3))]
        for c in range(pa, 4):
            ats[0].q[c] = q_s[:, c * 128:(c + 1) * 128] + qhalf(1, c)
        qt(1, [0, 1, 2, 3])
        qt(2, [0, 1, 2, 3])
        wait(cp_wqkv[1])
        perm_qkv(1)
        qt(3, [0, 1])
        qt(0, [4, 5, 6, 7])
        qt(1, [4, 5, 6, 7])
        ats[0].qk_all()
        qt(3, [2, 3])
        qt(2, [4, 5, 6, 7])
        for c in range(pb):
            ats[1].qk(c)
        qt(3, [4, 5])
        for c in sorted(ats[1].half):
            ats[1].qkb(c)
        wait(cp_wqkv[2], cp_wo, cp_b1, cp_b2)
        perm_qkv(2)
        for k_, fn_ in enumerate(perm_wo_pieces()):
            tl.trigger(tl.slot + wodl[0] + (k_ * wodl[1]) // 32, lambda piece, fn_=fn_: fn_())
        b1_p[:, 1280:FP] = jnp.zeros((1, 128), f32)
        b1_p[:, 0:F] = b1_v[...].astype(f32).reshape(1, F)
        b2_p[...] = b2_v[...].astype(f32).reshape(1, D)
        qt(3, [6, 7])
        for c in range(pb, NC):
            ats[1].qk(c)
        ats[2].start_at(rel([2, 3, 4, 5, 6, 7, 8, 9]))
        qt(0, [8, 9, 10, 11])
        ats[0].due_at(rel([3, 4, 4, 5, 6, 6, 7, 7]))
        qt(1, [8, 9, 10, 11])
        ats[1].due_at(rel([4, 5, 5, 6, 6, 7, 7, 99]))
        qt(2, [8, 9, 10, 11])
        halo(0, PB + P * M)
        qt(3, [8, 9, 10, 11])
        for c in sorted(ats[2].half):
            ats[2].qkb(c)
        wait(cp_w1)
        ats[2].due_at(rel([3, 4, 4, 5, 6, 6, 7, 7]))
        wblk(0)
        wblk(1)
        wblk(2)
        y0 = ln2(xs[0])
        h0 = mm_M1(y0, repack=True)
        h1 = mm_M1(ln2(xs[1]))
        h2 = mm_M1(ln2(xs[2]))
        wait(cp_w2)
        st = State()
        x0 = mm_M2(xs[0], h0, repack=True)
        x1 = mm_M2(xs[1], h1)
        at0 = mm_Q(ln1(x0), 1, first=True, nb_=nb, dl_=(4, 5, 6, 7, 8, 9, 10, 11), row0=PB)
        halo(1, PB + M)
        at1 = mm_Q(ln1(x1), 1, nb_=nb, dl_=(7, 8, 9, 10, 11, 12, 13, 14))
        x0 = mm_W(x0, at0.done())
        st.x1 = mm_M2(xs[2], h2)
        h0 = mm_M1(ln2(x0))
        st.x2 = mm_W(x1, at1.done())
        halo(1, HALO + M)
        st.y2 = ln2s(st.x2)
        put_out(0, mm_M2(x0, h0))
        st.at = ats[3]
        st.save()

        cp_xr.wait()
        scope("loop")
        assert (NB - NTAIL - P) % U == 0

        def body(i, carry):
            st = State()
            st.load()
            for u in range(U):
                step(st, P + i * U + u, last_in_block=(u == U - 1))
            st.save()
            return carry
        lax.fori_loop(0, (NB - NTAIL - P) // U, body, 0)

        scope("epi")
        st = State()
        st.load()
        for n in range(NB - NTAIL, NB):
            step(st, n)
        at = mm_Q(ln1(st.x1), 1, nb_=nb, dl_=edl)
        h2 = mm_M1(st.y2)
        put_out(NB - 2, mm_M2(st.x2, h2, js=(0, 1)))
        x3 = mm_W(st.x1, at.done())
        put_out(NB - 2, mm_M2(st.x2, h2, js=(2, 3)), 256)
        h3 = mm_M1(ln2(x3))
        if esplit == 2:
            put_out(NB - 1, mm_M2(x3, h3, js=(0, 1)))
            put_out(NB - 1, mm_M2(x3, h3, js=(2, 3)), 256)
        elif esplit == 4:
            for j in range(4):
                put_out(NB - 1, mm_M2(x3, h3, js=(j,)), j * 128)
        else:
            put_out(NB - 1, mm_M2(x3, h3))
        scope("outwait")
        pltpu.make_async_copy(o_v, o_hbm, osem).wait()
        scope(None)

    return kernel


def build(M=128, RC=16, RA=16, scopes=False, U=2, NTAIL=1, lag=1, nb0=(0, 0, 1, 1, 2, 2, 3, 3), wodl=(2, 15), pa=2, pb=8, edl=(8, 9, 10, 12, 13, 14, 15, 16), esplit=4, gd=0, gs=1, gx=0,
          nb=(-5, -5, -4, -4, -3, -3, -2, -2), dl=(14, 15, 16, 17, 18, 19, 20, 21)):
    @jax.jit
    def fn(A_x, A_wqkv, A_wo, B_x, B_w1, B_b1, B_w2, B_b2):
        x = A_x.reshape(S, D)
        anyspec = pl.BlockSpec(memory_space=pl.ANY)
        out = pl.pallas_call(
            make_kernel(M, RC, RA, scopes, U, NTAIL, nb, dl, lag, nb0, wodl, pa, pb, edl, esplit, gd, gs, gx),
            in_specs=[anyspec] * 7,
            out_specs=anyspec,
            out_shape=jax.ShapeDtypeStruct((S, D), bf16),
            scratch_shapes=[
                pltpu.VMEM((S, D), bf16), pltpu.VMEM((S, D), bf16),
                pltpu.VMEM((D, 3 * D), bf16), pltpu.VMEM((D, D), bf16),
                pltpu.VMEM((FP, D), bf16), pltpu.VMEM((FP, D), bf16),
                pltpu.VMEM((F,), bf16), pltpu.VMEM((D,), bf16),
                pltpu.VMEM((D // 2, 3 * D), u32), pltpu.VMEM((D // 2, D), u32),
                pltpu.VMEM((FP // 2, D), u32), pltpu.VMEM((FP // 2, D), u32),
                pltpu.VMEM((1, FP), f32), pltpu.VMEM((1, D), f32), pltpu.VMEM((4, H * WS, 128), f32),
                pltpu.VMEM((16, 4 * M + 2 * HALO, 128), f32),
                pltpu.VMEM((M // 2, D), u32), pltpu.VMEM((M, D), f32), pltpu.VMEM((M, D), f32), pltpu.VMEM((M, D), f32),
                pltpu.VMEM((8, 128), u32),
                pltpu.SemaphoreType.DMA((12,)), pltpu.SemaphoreType.DMA(()),
            ],
            compiler_params=pltpu.CompilerParams(vmem_limit_bytes=100 << 20),
        )(x, A_wqkv, A_wo, B_w1.T, B_b1, B_w2, B_b2)
        return out.reshape(1, S, D)
    return fn


pallas_interleave_layers__sliding_local_dilated__mixer_channel_mlp__prompt_kernel = build()
```

```python
import functools
import math

import jax
import jax.numpy as jnp
import numpy as np
from jax import lax
import jax.experimental.pallas as pl
import jax.experimental.pallas.tpu as pltpu

S, D, F = 2048, 512, 1376
FP = 1408
H, DH, W, DIL = 32, 16, 8, 2
HALO = 16
WS = 20
EPS = 1e-5
LOG2E = 1.4426950408889634
QSCALE = (DH ** -0.5) * LOG2E
QSCALE_BITS = int(np.float32(QSCALE).view(np.uint32))
NEG = -1e9 * LOG2E
f32, bf16, u32 = jnp.float32, jnp.bfloat16, jnp.uint32

M = 128
NB = S // M
RC = 16
RA = 16
NC = M // RA
P = 3
U = 2
PB = 2 * HALO + M

NB_SLOTS = (-5, -5, -4, -4, -3, -3, -2, -2)
DL_SLOTS = (15, 16, 17, 18, 19, 20, 21, 22)
DL_LAST = (14, 15, 16, 17, 18, 19, 20, 21)
DL_TAIL = (8, 9, 10, 12, 13, 14, 15, 16)


def _ln(x):
    m = jnp.mean(x, axis=-1, keepdims=True)
    xc = x - m
    v = jnp.mean(xc * xc, axis=-1, keepdims=True)
    return xc * lax.rsqrt(v + EPS)


def _gelu(x):
    c = math.sqrt(2.0 / math.pi)
    inner = x * (c + (c * 0.044715) * (x * x))
    return (0.5 * x) * (1.0 + jnp.tanh(inner))


def _dot(a, b):
    return jnp.dot(a, b, preferred_element_type=f32)


def _dot_t(a, b):
    return lax.dot_general(a, b, (((1,), (1,)), ((), ())), preferred_element_type=f32)


def _or_all(xs):
    return functools.reduce(lambda u, v: u | v, xs)


def _pieces(a):
    return [a[r:r + 8, c:c + 128] for r in range(0, a.shape[0], 8) for c in range(0, a.shape[1], 128)]


def _patch(wu, r, tok):
    rows = wu[r:r + 8]
    if wu.shape[1] > 128:
        rows = jnp.concatenate([rows[:, 0:128] | tok, rows[:, 128:]], axis=1)
    else:
        rows = rows | tok
    parts = ([wu[:r]] if r > 0 else []) + [rows] + ([wu[r + 8:]] if r + 8 < wu.shape[0] else [])
    return jnp.concatenate(parts, axis=0)


class _Timeline:
    def __init__(self):
        self.slot, self.due, self.trig = 0, {}, {}

    def rel(self, offs):
        return [self.slot + o for o in offs]

    def deadline(self, slot, fn):
        self.due.setdefault(slot, []).append(fn)

    def trigger(self, slot, fn):
        self.trig.setdefault(slot, []).append(fn)

    def weights(self, wu, r=0, off=0):
        for fn in self.due.pop(self.slot + off, []):
            wu = _patch(wu, r, fn())
        return wu

    def done(self, r, n=1):
        lo = self.slot
        self.slot += n
        for s in range(lo, self.slot):
            for fn in self.trig.pop(s, []):
                fn(r[r.shape[0] - 8:, 0:128])

    def barrier(self):
        assert not self.trig
        self.due.clear()


def _kernel(x_hbm, wqkv_hbm, wo_hbm, w1t_hbm, b1_hbm, w2_hbm, b2_hbm, o_hbm,
            x_v, o_v, wqkv_v, wo_v, w1_v, w2_v, b1_v, b2_v,
            wqkv_p, wo_p, w1_p, w2_p, b1_p, b2_p, wo_tmp, kv, o_s, q_s, x1_s, zero_s, sems, osem):
    tl = _Timeline()

    XE = (P + 1) * M
    cp = pltpu.make_async_copy
    cp_x0 = cp(x_hbm.at[0:M], x_v.at[0:M], sems.at[0])
    cp_wq = [cp(wqkv_hbm.at[hf * 256:(hf + 1) * 256, 0:D], wqkv_v.at[hf * 256:(hf + 1) * 256, 0:D], sems.at[1 + hf])
             for hf in range(2)]
    cp_x123 = cp(x_hbm.at[M:XE], x_v.at[M:XE], sems.at[3])
    cp_wk = cp(wqkv_hbm.at[:, D:2 * D], wqkv_v.at[:, D:2 * D], sems.at[4])
    cp_wv = cp(wqkv_hbm.at[:, 2 * D:3 * D], wqkv_v.at[:, 2 * D:3 * D], sems.at[5])
    cp_wo = cp(wo_hbm, wo_v, sems.at[6])
    cp_b1 = cp(b1_hbm, b1_v, sems.at[7])
    cp_b2 = cp(b2_hbm, b2_v, sems.at[8])
    cp_w1 = cp(w1t_hbm, w1_v.at[0:F], sems.at[9])
    cp_w2 = cp(w2_hbm, w2_v.at[0:F], sems.at[10])
    cp_xr = cp(x_hbm.at[XE:S], x_v.at[XE:S], sems.at[11])
    for c_ in [cp_x0, cp_wq[0], cp_wq[1], cp_x123, cp_wk, cp_wv, cp_wo, cp_b1, cp_b2, cp_w1, cp_w2, cp_xr]:
        c_.start()

    def wait(*cps):
        tl.barrier()
        for c_ in cps:
            c_.wait()

    def rowslice(n):
        r = n * M
        if not isinstance(n, int):
            r = pl.multiple_of(r, M)
        return pl.ds(r, M)

    lane = lax.broadcasted_iota(jnp.int32, (8, 128), 1)
    dq = (lane % 16) // 4
    g_, j_, h_ = lane // 32, (lane % 32) // 8, lane % 8
    idx = [h_ * 16 + 4 * ((i + j_) % 4) + g_ for i in range(4)]
    msk = [dq == t for t in range(4)]

    def perm_qkv(t, rows=range(D // 16)):
        for i in range(4):
            for r in rows:
                src = [pltpu.bitcast(wqkv_v[r * 16:(r + 1) * 16, t * D + j * 128: t * D + (j + 1) * 128], u32)
                       for j in range(4)]
                m = src[(0 - i) % 4]
                for tq in range(1, 4):
                    m = jnp.where(msk[tq], src[(tq - i) % 4], m)
                wqkv_p[r * 8:(r + 1) * 8, t * D + i * 128: t * D + (i + 1) * 128] = \
                    jnp.take_along_axis(m, idx[i], axis=1)

    def perm_wo_a(cb, j):
        for hh in range(8 * j, 8 * j + 8):
            wo_tmp[cb, hh * WS:hh * WS + DH, :] = wo_v[hh * DH:(hh + 1) * DH, cb * 128:(cb + 1) * 128].astype(f32)

    def perm_wo_b(cb, i):
        for g in range(4):
            rows = [wo_tmp[cb, pl.ds(j * 8 * WS + 4 * ((i + j) % 4) + g, 8, stride=WS), :] for j in range(4)]
            r0 = (i * 128 + g * 32) // 2
            wo_p[r0:r0 + 16, cb * 128:(cb + 1) * 128] = \
                pltpu.bitcast(jnp.concatenate(rows, axis=0).astype(bf16), u32)

    def ztok(pieces):
        return _or_all([pltpu.bitcast(p, u32) for p in pieces]) & zero_s[...]

    def rows_map(fn, x):
        return jnp.concatenate([fn(x[r:r + RC]) for r in range(0, x.shape[0], RC)], axis=0)

    def ln1(x):
        return rows_map(_ln, x).astype(bf16)

    def ln2(x):
        return rows_map(lambda a: _ln(_ln(a)), x).astype(bf16)

    def halo(layer, end):
        L = layer * 8
        kv[L:L + 8, 0:HALO, :] = kv[L:L + 8, end - HALO:end, :]

    class Attn:
        def __init__(self, layer, first=False, row0=HALO):
            self.layer, self.first, self.row0 = layer, first, row0
            self.q = [None] * 4
            self.half, self.logit, self.outs, self.timed = {}, {}, {}, set()

        def qk(self, c, tok=None):
            L, r0 = self.layer * 8, c * RA
            g0 = self.row0 + r0
            if tok is None:
                sc = QSCALE
            else:
                sc = jnp.concatenate([pltpu.bitcast(tok | QSCALE_BITS, f32)] * (RA // 8), axis=0)
            qs = [self.q[j][r0:r0 + RA] * sc for j in range(4)]
            ls = []
            for w in range(W):
                s = None
                for j in range(4):
                    t = qs[j] * kv[L + j, pl.ds(g0 - DIL * w, RA), :]
                    s = t if s is None else s + t
                ls.append(s)
            self.half[c] = [s + pltpu.roll(s, 64, 1) for s in ls]
            for c2 in sorted(self.half):
                if c2 < c:
                    self.qkb(c2)

        def qkb(self, c):
            r0 = c * RA
            ls = [s + pltpu.roll(s, 32, 1) for s in self.half.pop(c)]
            if self.first and r0 < HALO:
                row = r0 + lax.broadcasted_iota(jnp.int32, (RA, 128), 0)
                ls = [ls[0]] + [jnp.where(row >= DIL * w, ls[w], NEG) for w in range(1, W)]
            self.logit[c] = ls

        def flush(self):
            for c in sorted(self.half):
                self.qkb(c)

        def qk_all(self):
            for c in range(NC):
                self.qk(c)
            self.flush()

        def av(self, c):
            L, r0 = self.layer * 8, c * RA
            g0 = self.row0 + r0
            ls = self.logit[c]
            m = ls[0]
            for w in range(1, W):
                m = jnp.maximum(m, ls[w])
            ps = [jnp.exp2(l - m) for l in ls]
            den = ps[0]
            for w in range(1, W):
                den = den + ps[w]
            inv = 1.0 / den
            oj = []
            for j in range(4):
                a = None
                for w in range(W):
                    t = ps[w] * kv[L + 4 + j, pl.ds(g0 - DIL * w, RA), :]
                    a = t if a is None else a + t
                oj.append(a * inv)
            self.outs[c] = jnp.concatenate(oj, axis=1)

        def finish(self, c):
            assert c in self.logit or c in self.half
            if c in self.half:
                self.qkb(c)
            if c not in self.outs:
                self.av(c)

        def start_at(self, slots):
            for c, s in enumerate(slots):
                tl.trigger(s, lambda piece, c=c: self.qk(c, ztok([piece])))

        def due_at(self, slots):
            def tok(c):
                self.finish(c)
                return ztok(_pieces(self.outs[c]))
            for c, s in enumerate(slots):
                tl.deadline(s, lambda c=c: tok(c))

        def done(self):
            for c in range(NC):
                self.finish(c)
            return jnp.concatenate([self.outs[c] for c in range(NC)], axis=0).astype(bf16)

    def q_tile(at, y, c):
        wu = tl.weights(wqkv_p[:, c * 128:(c + 1) * 128])
        r = _dot(y, pltpu.bitcast(wu, bf16))
        if c < 4:
            at.q[c] = r
        else:
            kv[at.layer * 8 + c - 4, at.row0:at.row0 + M, :] = r
        tl.done(r)

    def mm_Q(y, layer, dl, first=False, row0=HALO):
        at = Attn(layer, first=first, row0=row0)
        end = tl.slot + 12
        at.start_at([end + s for s in NB_SLOTS])
        at.due_at([end + s for s in dl])
        for c in range(12):
            q_tile(at, y, c)
        return at

    def mm_W(x, o):
        outs = []
        for j in range(4):
            cs = slice(j * 128, (j + 1) * 128)
            r = _dot(o, pltpu.bitcast(tl.weights(wo_p[:, cs]), bf16))
            tl.done(r)
            outs.append(x[:, cs] + r)
        return jnp.concatenate(outs, axis=1)

    def mm_M1(y, repack=False):
        hs = []
        for t in range(FP // 128):
            n0 = t * 128
            if repack:
                wu = pltpu.bitcast(w1_v[n0:n0 + 128, :], u32)
                w1_p[n0 // 2:n0 // 2 + 64, :] = wu
            else:
                wu = w1_p[n0 // 2:n0 // 2 + 64, :]
            r = _dot_t(y, pltpu.bitcast(tl.weights(wu), bf16))
            tl.done(r)
            hs.append(_gelu(r + b1_p[:, n0:n0 + 128]))
        return jnp.concatenate(hs, axis=1).astype(bf16)

    def mm_M2(x, h, repack=False, js=(0, 1, 2, 3)):
        outs = []
        for j in js:
            cs = slice(j * 128, (j + 1) * 128)
            if repack:
                wu = pltpu.bitcast(w2_v[:, cs], u32)
                w2_p[:, cs] = wu
            else:
                wu = w2_p[:, cs]
            ps = [p for p in range(11) if (4 * p) // 11 == j]
            for i, p in enumerate(ps):
                wu = tl.weights(wu, ((4 * p) % 11) * 64, off=i)
            r = _dot(h, pltpu.bitcast(wu, bf16))
            tl.done(r, len(ps))
            outs.append(x[:, cs] + r + b2_p[:, cs])
        return jnp.concatenate(outs, axis=1)

    def xblk(n):
        return x_v[rowslice(n), :].astype(f32)

    def put_out(n, val, c0=0):
        cs = slice(c0, c0 + val.shape[1])
        o_v[rowslice(n), cs] = val.astype(bf16)
        cp(o_v.at[rowslice(n), cs], o_hbm.at[rowslice(n), cs], osem).start()

    def save(o, x1):
        x1_s[...] = x1
        o_s[...] = pltpu.bitcast(o, u32)
        tl.barrier()

    def load():
        return pltpu.bitcast(o_s[...], bf16), x1_s[...]

    def step_a(o, x1, n):
        x = mm_W(xblk(n), o)
        y = ln2(x)
        at = mm_Q(ln1(x1), 1, DL_SLOTS)
        h = mm_M1(y)
        x1n = mm_M2(x, h)
        x2 = mm_W(x1, at.done())
        halo(1, HALO + M)
        return x1n, x2

    def step(o, x1, n, last):
        x1n, x2 = step_a(o, x1, n)
        y2 = ln2(x2)
        at = mm_Q(ln1(xblk(n + 1)), 0, DL_LAST if last else DL_SLOTS)
        h2 = mm_M1(y2)
        put_out(n - 1, mm_M2(x2, h2))
        on = at.done()
        halo(0, HALO + M)
        return on, x1n

    kv[:, PB - HALO:PB, :] = jnp.zeros((16, HALO, 128), f32)
    zero_s[...] = jnp.zeros((8, 128), u32)
    w1_v[F:FP, :] = jnp.zeros((FP - F, D), bf16)
    w2_v[F:FP, :] = jnp.zeros((FP - F, D), bf16)
    ats = [Attn(0, first=(b == 0), row0=PB + b * M) for b in range(P)] + [Attn(0)]

    def qt(b, cs):
        for c in cs:
            q_tile(ats[b], ys[b], c)

    def wblk(b):
        xs[b] = mm_W(xs[b], ats[b].done())

    def qhalf(hf, c):
        w = pltpu.bitcast(wqkv_p[hf * 128:(hf + 1) * 128, c * 128:(c + 1) * 128], bf16)
        return _dot(ys[0][:, hf * 256:(hf + 1) * 256], w)

    wait(cp_x0)
    xs = [xblk(0)]
    ys = [ln1(xs[0])]
    wait(cp_wq[0])
    perm_qkv(0, rows=range(0, 16))
    for c in range(4):
        q_s[:, c * 128:(c + 1) * 128] = qhalf(0, c)
    wait(cp_wq[1])
    perm_qkv(0, rows=range(16, 32))
    for c in range(2):
        ats[0].q[c] = q_s[:, c * 128:(c + 1) * 128] + qhalf(1, c)
    wait(cp_x123)
    xs += [xblk(1), xblk(2)]
    ys += [ln1(xs[1]), ln1(xs[2]), ln1(xblk(3))]
    for c in range(2, 4):
        ats[0].q[c] = q_s[:, c * 128:(c + 1) * 128] + qhalf(1, c)
    qt(1, [0, 1, 2, 3])
    qt(2, [0, 1, 2, 3])
    wait(cp_wk)
    perm_qkv(1)
    qt(3, [0, 1])
    qt(0, [4, 5, 6, 7])
    qt(1, [4, 5, 6, 7])
    ats[0].qk_all()
    qt(3, [2, 3])
    qt(2, [4, 5, 6, 7])
    for c in range(NC):
        ats[1].qk(c)
    qt(3, [4, 5])
    ats[1].flush()
    wait(cp_wv, cp_wo, cp_b1, cp_b2)
    perm_qkv(2)
    wo_pieces = [functools.partial(fn, cb, t) for cb in range(4) for fn in (perm_wo_a, perm_wo_b) for t in range(4)]
    for k, fn in enumerate(wo_pieces):
        tl.trigger(tl.slot + 1 + (k * 11) // 32, lambda piece, fn=fn: fn())
    b1_p[:, 1280:FP] = jnp.zeros((1, 128), f32)
    b1_p[:, 0:F] = b1_v[...].astype(f32).reshape(1, F)
    b2_p[...] = b2_v[...].astype(f32).reshape(1, D)
    qt(3, [6, 7])
    qt(0, [8, 9, 10, 11])
    ats[0].due_at(tl.rel((3, 4, 4, 5, 6, 6, 7, 7)))
    qt(1, [8, 9, 10, 11])
    qt(2, [8, 9, 10, 11])
    halo(0, PB + P * M)
    ats[1].due_at(tl.rel((0, 1, 2, 3, 4, 5, 6, 7)))
    wblk(0)
    qt(3, [8, 9, 10, 11])
    y0 = ln2(xs[0])
    wait(cp_w1)
    ats[2].qk_all()
    ats[2].due_at(tl.rel((7, 8, 9, 10, 11, 12, 13, 14)))
    h0 = mm_M1(y0, repack=True)
    wblk(1)
    wblk(2)
    h1 = mm_M1(ln2(xs[1]))
    h2 = mm_M1(ln2(xs[2]))
    wait(cp_w2)
    x0 = mm_M2(xs[0], h0, repack=True)
    x1 = mm_M2(xs[1], h1)
    at0 = mm_Q(ln1(x0), 1, (4, 5, 6, 7, 8, 9, 10, 11), first=True, row0=PB)
    halo(1, PB + M)
    at1 = mm_Q(ln1(x1), 1, (7, 8, 9, 10, 11, 12, 13, 14))
    x0 = mm_W(x0, at0.done())
    x2 = mm_M2(xs[2], h2)
    h0 = mm_M1(ln2(x0))
    x1 = mm_W(x1, at1.done())
    halo(1, HALO + M)
    ats[3].start_at(tl.rel((0, 1, 2, 3, 4, 5, 6, 7)))
    put_out(0, mm_M2(x0, h0))
    ats[3].due_at(tl.rel(DL_LAST))
    h1 = mm_M1(ln2(x1))
    put_out(1, mm_M2(x1, h1))
    o3 = ats[3].done()
    halo(0, HALO + M)
    save(o3, x2)

    wait(cp_xr)

    def body(i, carry):
        o, x1 = load()
        for u in range(U):
            o, x1 = step(o, x1, P + i * U + u, last=(u == U - 1))
        save(o, x1)
        return carry
    lax.fori_loop(0, (NB - 1 - P) // U, body, 0)

    o, x1 = load()
    x1, x2 = step_a(o, x1, NB - 1)
    y2 = ln2(x2)
    at = mm_Q(ln1(x1), 1, DL_TAIL)
    h2 = mm_M1(y2)
    put_out(NB - 2, mm_M2(x2, h2, js=(0, 1)))
    x3 = mm_W(x1, at.done())
    put_out(NB - 2, mm_M2(x2, h2, js=(2, 3)), 256)
    h3 = mm_M1(ln2(x3))
    for j in range(4):
        put_out(NB - 1, mm_M2(x3, h3, js=(j,)), j * 128)
    cp(o_v, o_hbm, osem).wait()


@jax.jit
def pallas_interleave_layers__sliding_local_dilated__mixer_channel_mlp__prompt_kernel(
    A_x: jax.Array,
    A_wqkv: jax.Array,
    A_wo: jax.Array,
    B_x: jax.Array,
    B_w1: jax.Array,
    B_b1: jax.Array,
    B_w2: jax.Array,
    B_b2: jax.Array,
):
    assert (NB - 1 - P) % U == 0
    anyspec = pl.BlockSpec(memory_space=pl.ANY)
    out = pl.pallas_call(
        _kernel,
        in_specs=[anyspec] * 7,
        out_specs=anyspec,
        out_shape=jax.ShapeDtypeStruct((S, D), bf16),
        scratch_shapes=[
            pltpu.VMEM((S, D), bf16), pltpu.VMEM((S, D), bf16),
            pltpu.VMEM((D, 3 * D), bf16), pltpu.VMEM((D, D), bf16),
            pltpu.VMEM((FP, D), bf16), pltpu.VMEM((FP, D), bf16),
            pltpu.VMEM((F,), bf16), pltpu.VMEM((D,), bf16),
            pltpu.VMEM((D // 2, 3 * D), u32), pltpu.VMEM((D // 2, D), u32),
            pltpu.VMEM((FP // 2, D), u32), pltpu.VMEM((FP // 2, D), u32),
            pltpu.VMEM((1, FP), f32), pltpu.VMEM((1, D), f32),
            pltpu.VMEM((4, H * WS, 128), f32),
            pltpu.VMEM((16, 4 * M + 2 * HALO, 128), f32),
            pltpu.VMEM((M // 2, D), u32), pltpu.VMEM((M, D), f32),
            pltpu.VMEM((M, D), f32),
            pltpu.VMEM((8, 128), u32),
            pltpu.SemaphoreType.DMA((12,)), pltpu.SemaphoreType.DMA(()),
        ],
        compiler_params=pltpu.CompilerParams(vmem_limit_bytes=100 << 20),
    )(A_x.reshape(S, D), A_wqkv, A_wo, B_w1.T, B_b1, B_w2, B_b2)
    return out.reshape(1, S, D)
```

```python
import functools
import math

import jax
import jax.numpy as jnp
import numpy as np
from jax import lax
import jax.experimental.pallas as pl
import jax.experimental.pallas.tpu as pltpu

S, D, F = 2048, 512, 1376
FP = 1408
H, DH, W, DIL = 32, 16, 8, 2
HALO = 16
WS = 20
EPS = 1e-5
LOG2E = 1.4426950408889634
QSCALE = (DH ** -0.5) * LOG2E
QSCALE_BITS = int(np.float32(QSCALE).view(np.uint32))
NEG = -1e9 * LOG2E
f32, bf16, u32 = jnp.float32, jnp.bfloat16, jnp.uint32

M = 128
NB = S // M
RC = 16
RA = 16
NC = M // RA
P = 3
U = 2
PB = 2 * HALO + M

NB_SLOTS = (-5, -4, -3, -2, -1, 0, 1, 2)
DL_SLOTS = (15, 16, 17, 18, 19, 20, 21, 22)
DL_LAST = (14, 15, 16, 17, 18, 19, 20, 21)
DL_TAIL = (8, 9, 10, 12, 13, 14, 15, 16)
M1_ORDER = (0, 1, 2, 3, 10, 4, 5, 6, 7, 8, 9)


def _ln(x):
    m = jnp.mean(x, axis=-1, keepdims=True)
    xc = x - m
    v = jnp.mean(xc * xc, axis=-1, keepdims=True)
    return xc * lax.rsqrt(v + EPS)


def _ln_half(x):
    m = jnp.mean(x, axis=-1, keepdims=True)
    xc = x - m
    v4 = jnp.sum(xc * xc, axis=-1, keepdims=True) * (4.0 / D)
    return xc * lax.rsqrt(v4 + 4.0 * EPS)


def _gelu_from_half(z):
    c = math.sqrt(2.0 / math.pi)
    inner = z * (2.0 * c + (8.0 * c * 0.044715) * (z * z))
    return z + z * jnp.tanh(inner)


def _dot(a, b):
    return jnp.dot(a, b, preferred_element_type=f32)


def _dot_t(a, b):
    return lax.dot_general(a, b, (((1,), (1,)), ((), ())), preferred_element_type=f32)


def _or_all(xs):
    return functools.reduce(lambda u, v: u | v, xs)


def _pieces(a):
    return [a[r:r + 8, c:c + 128] for r in range(0, a.shape[0], 8) for c in range(0, a.shape[1], 128)]


def _patch(wu, r, tok):
    rows = wu[r:r + 8]
    if wu.shape[1] > 128:
        rows = jnp.concatenate([rows[:, 0:128] | tok, rows[:, 128:]], axis=1)
    else:
        rows = rows | tok
    parts = ([wu[:r]] if r > 0 else []) + [rows] + ([wu[r + 8:]] if r + 8 < wu.shape[0] else [])
    return jnp.concatenate(parts, axis=0)


class _Timeline:
    def __init__(self):
        self.slot, self.due, self.trig = 0, {}, {}

    def rel(self, offs):
        return [self.slot + o for o in offs]

    def deadline(self, slot, fn):
        self.due.setdefault(slot, []).append(fn)

    def trigger(self, slot, fn):
        self.trig.setdefault(slot, []).append(fn)

    def weights(self, wu, r=0, off=0):
        for fn in self.due.pop(self.slot + off, []):
            wu = _patch(wu, r, fn())
        return wu

    def done(self, r, n=1):
        lo = self.slot
        self.slot += n
        for s in range(lo, self.slot):
            for fn in self.trig.pop(s, []):
                fn(r[r.shape[0] - 8:, 0:128])

    def barrier(self):
        assert not self.trig
        self.due.clear()


def _kernel(x_hbm, wqkv_hbm, wo_hbm, w1t_hbm, b1_hbm, w2_hbm, b2_hbm, o_hbm,
            x_v, o_v, wqkv_v, wo_v, w1_v, w2_v, b1_v, b2_v,
            wqkv_p, wo_p, w1_p, w2_p, b1_p, wo_tmp, kv, o_s, q_s, x1_s, zero_s, sems, osem):
    tl = _Timeline()

    XE = (P + 1) * M
    cp = pltpu.make_async_copy
    cp_x0 = cp(x_hbm.at[0:M], x_v.at[0:M], sems.at[0])
    cp_wq = [cp(wqkv_hbm.at[hf * 256:(hf + 1) * 256, 0:D], wqkv_v.at[hf * 256:(hf + 1) * 256, 0:D], sems.at[1 + hf])
             for hf in range(2)]
    cp_x123 = cp(x_hbm.at[M:XE], x_v.at[M:XE], sems.at[3])
    cp_wk = cp(wqkv_hbm.at[:, D:2 * D], wqkv_v.at[:, D:2 * D], sems.at[4])
    cp_wv = cp(wqkv_hbm.at[:, 2 * D:3 * D], wqkv_v.at[:, 2 * D:3 * D], sems.at[5])
    cp_wo = cp(wo_hbm, wo_v, sems.at[6])
    cp_b1 = cp(b1_hbm, b1_v, sems.at[7])
    cp_b2 = cp(b2_hbm, b2_v, sems.at[8])
    cp_w1 = cp(w1t_hbm, w1_v, sems.at[9])
    cp_w2 = cp(w2_hbm, w2_v.at[0:F], sems.at[10])
    cp_xr = cp(x_hbm.at[XE:S], x_v.at[XE:S], sems.at[11])
    for c_ in [cp_x0, cp_wq[0], cp_wq[1], cp_x123, cp_wk, cp_wv, cp_wo, cp_b1, cp_b2, cp_w1, cp_w2, cp_xr]:
        c_.start()

    def wait(*cps):
        tl.barrier()
        for c_ in cps:
            c_.wait()

    def rowslice(n):
        r = n * M
        if not isinstance(n, int):
            r = pl.multiple_of(r, M)
        return pl.ds(r, M)

    lane = lax.broadcasted_iota(jnp.int32, (8, 128), 1)
    dq = (lane % 16) // 4
    g_, j_, h_ = lane // 32, (lane % 32) // 8, lane % 8
    idx = [h_ * 16 + 4 * ((i + j_) % 4) + g_ for i in range(4)]
    msk = [dq == t for t in range(4)]

    def perm_qkv(t, rows=range(D // 16)):
        for i in range(4):
            for r in rows:
                src = [pltpu.bitcast(wqkv_v[r * 16:(r + 1) * 16, t * D + j * 128: t * D + (j + 1) * 128], u32)
                       for j in range(4)]
                m = src[(0 - i) % 4]
                for tq in range(1, 4):
                    m = jnp.where(msk[tq], src[(tq - i) % 4], m)
                wqkv_p[r * 8:(r + 1) * 8, t * D + i * 128: t * D + (i + 1) * 128] = \
                    jnp.take_along_axis(m, idx[i], axis=1)

    def perm_wo_a(cb, j):
        for hh in range(8 * j, 8 * j + 8):
            wo_tmp[cb, hh * WS:hh * WS + DH, :] = wo_v[hh * DH:(hh + 1) * DH, cb * 128:(cb + 1) * 128].astype(f32)

    def perm_wo_b(cb, i):
        for g in range(4):
            rows = [wo_tmp[cb, pl.ds(j * 8 * WS + 4 * ((i + j) % 4) + g, 8, stride=WS), :] for j in range(4)]
            r0 = (i * 128 + g * 32) // 2
            wo_p[r0:r0 + 16, cb * 128:(cb + 1) * 128] = \
                pltpu.bitcast(jnp.concatenate(rows, axis=0).astype(bf16), u32)

    def ztok(pieces):
        return _or_all([pltpu.bitcast(p, u32) for p in pieces]) & zero_s[...]

    def rows_map(fn, x):
        return jnp.concatenate([fn(x[r:r + RC]) for r in range(0, x.shape[0], RC)], axis=0)

    def ln1(x):
        return rows_map(_ln, x).astype(bf16)

    def ln2(x):
        return rows_map(lambda a: _ln_half(_ln(a)), x).astype(bf16)

    def halo(layer, end):
        L = layer * 8
        kv[L:L + 8, 0:HALO, :] = kv[L:L + 8, end - HALO:end, :]

    class Attn:
        def __init__(self, layer, first=False, row0=HALO):
            self.layer, self.first, self.row0 = layer, first, row0
            self.q = [None] * 4
            self.half, self.logit, self.outs, self.timed = {}, {}, {}, set()

        def qk(self, c, tok=None):
            L, r0 = self.layer * 8, c * RA
            g0 = self.row0 + r0
            if tok is None:
                sc = QSCALE
            else:
                sc = jnp.concatenate([pltpu.bitcast(tok | QSCALE_BITS, f32)] * (RA // 8), axis=0)
            qs = [self.q[j][r0:r0 + RA] * sc for j in range(4)]
            ls = []
            for w in range(W):
                s = None
                for j in range(4):
                    t = qs[j] * kv[L + j, pl.ds(g0 - DIL * w, RA), :]
                    s = t if s is None else s + t
                ls.append(s)
            self.half[c] = [s + pltpu.roll(s, 64, 1) for s in ls]
            for c2 in sorted(self.half):
                if c2 < c:
                    self.qkb(c2)

        def qkb(self, c):
            r0 = c * RA
            ls = [s + pltpu.roll(s, 32, 1) for s in self.half.pop(c)]
            if self.first and r0 < HALO:
                row = r0 + lax.broadcasted_iota(jnp.int32, (RA, 128), 0)
                ls = [ls[0]] + [jnp.where(row >= DIL * w, ls[w], NEG) for w in range(1, W)]
            self.logit[c] = ls

        def flush(self):
            for c in sorted(self.half):
                self.qkb(c)

        def qk_all(self):
            for c in range(NC):
                self.qk(c)
            self.flush()

        def av(self, c):
            L, r0 = self.layer * 8, c * RA
            g0 = self.row0 + r0
            ls = self.logit[c]
            m = ls[0]
            for w in range(1, W):
                m = jnp.maximum(m, ls[w])
            ps = [jnp.exp2(l - m) for l in ls]
            den = ps[0]
            for w in range(1, W):
                den = den + ps[w]
            inv = pl.reciprocal(den, approx=True)
            inv = inv * (2.0 - den * inv)
            oj = []
            for j in range(4):
                a = None
                for w in range(W):
                    t = ps[w] * kv[L + 4 + j, pl.ds(g0 - DIL * w, RA), :]
                    a = t if a is None else a + t
                oj.append(a * inv)
            self.outs[c] = jnp.concatenate(oj, axis=1)

        def finish(self, c):
            assert c in self.logit or c in self.half
            if c in self.half:
                self.qkb(c)
            if c not in self.outs:
                self.av(c)

        def start_at(self, slots):
            for c, s in enumerate(slots):
                tl.trigger(s, lambda piece, c=c: self.qk(c, ztok([piece])))

        def due_at(self, slots):
            def tok(c):
                self.finish(c)
                return ztok(_pieces(self.outs[c]))
            for c, s in enumerate(slots):
                tl.deadline(s, lambda c=c: tok(c))

        def done(self):
            for c in range(NC):
                self.finish(c)
            return jnp.concatenate([self.outs[c] for c in range(NC)], axis=0).astype(bf16)

    def q_tile(at, y, c):
        wu = tl.weights(wqkv_p[:, c * 128:(c + 1) * 128])
        r = _dot(y, pltpu.bitcast(wu, bf16))
        if c < 4:
            at.q[c] = r
        else:
            kv[at.layer * 8 + c - 4, at.row0:at.row0 + M, :] = r
        tl.done(r)

    def mm_Q(y, layer, dl, first=False, row0=HALO):
        at = Attn(layer, first=first, row0=row0)
        end = tl.slot + 12
        at.start_at([end + s for s in NB_SLOTS])
        at.due_at([end + s for s in dl])
        for c in range(12):
            q_tile(at, y, c)
        return at

    def mm_W(x, o):
        outs = []
        for j in range(4):
            cs = slice(j * 128, (j + 1) * 128)
            r = _dot(o, pltpu.bitcast(tl.weights(wo_p[:, cs]), bf16))
            tl.done(r)
            outs.append(x[:, cs] + r)
        return jnp.concatenate(outs, axis=1)

    def mm_M1(y, repack=False):
        hs = {}
        for t in M1_ORDER:
            n0 = t * 128
            nr = min(128, F - n0)
            if repack:
                wu = pltpu.bitcast(w1_v[n0:n0 + nr, :], u32)
                w1_p[n0 // 2:(n0 + nr) // 2, :] = wu
            else:
                wu = w1_p[n0 // 2:(n0 + nr) // 2, :]
            w = pltpu.bitcast(tl.weights(wu), bf16)
            if nr == 128:
                r = _dot_t(y, w)
                tl.done(r)
            else:
                rt = _dot_t(w, y)
                tl.done(rt)
                r = jnp.concatenate([rt, jnp.zeros((128 - nr, M), f32)], axis=0).T
            hs[t] = _gelu_from_half(r + b1_p[:, n0:n0 + 128])
        return jnp.concatenate([hs[t] for t in range(FP // 128)], axis=1).astype(bf16)

    def mm_M2(x, h, repack=False, js=(0, 1, 2, 3)):
        outs = []
        for j in js:
            cs = slice(j * 128, (j + 1) * 128)
            if repack:
                wu = pltpu.bitcast(w2_v[:, cs], u32)
                w2_p[:, cs] = wu
            else:
                wu = w2_p[:, cs]
            ps = [p for p in range(11) if (4 * p) // 11 == j]
            for i, p in enumerate(ps):
                wu = tl.weights(wu, ((4 * p) % 11) * 64, off=i)
            r = _dot(h, pltpu.bitcast(wu, bf16))
            tl.done(r, len(ps))
            outs.append(x[:, cs] + r)
        return jnp.concatenate(outs, axis=1)

    def xblk(n):
        return x_v[rowslice(n), :].astype(f32)

    def put_out(n, val, c0=0):
        cs = slice(c0, c0 + val.shape[1])
        o_v[rowslice(n), cs] = val.astype(bf16)
        cp(o_v.at[rowslice(n), cs], o_hbm.at[rowslice(n), cs], osem).start()

    def save(o, x1):
        x1_s[...] = x1
        o_s[...] = pltpu.bitcast(o, u32)
        tl.barrier()

    def load():
        return pltpu.bitcast(o_s[...], bf16), x1_s[...]

    def step_a(o, x1, n):
        x = mm_W(xblk(n), o)
        y = ln2(x)
        at = mm_Q(ln1(x1), 1, DL_SLOTS)
        h = mm_M1(y)
        x1n = mm_M2(x, h)
        x2 = mm_W(x1, at.done())
        halo(1, HALO + M)
        return x1n, x2

    def step(o, x1, n, last):
        x1n, x2 = step_a(o, x1, n)
        y2 = ln2(x2)
        at = mm_Q(ln1(xblk(n + 1)), 0, DL_LAST if last else DL_SLOTS)
        h2 = mm_M1(y2)
        put_out(n - 1, mm_M2(x2, h2))
        on = at.done()
        halo(0, HALO + M)
        return on, x1n

    kv[:, PB - HALO:PB, :] = jnp.zeros((16, HALO, 128), f32)
    zero_s[...] = jnp.zeros((8, 128), u32)
    ats = [Attn(0, first=(b == 0), row0=PB + b * M) for b in range(P)] + [Attn(0)]

    def qt(b, cs):
        for c in cs:
            q_tile(ats[b], ys[b], c)

    def wblk(b):
        xs[b] = mm_W(xs[b], ats[b].done())

    def qhalf(hf, c):
        w = pltpu.bitcast(wqkv_p[hf * 128:(hf + 1) * 128, c * 128:(c + 1) * 128], bf16)
        return _dot(ys[0][:, hf * 256:(hf + 1) * 256], w)

    wait(cp_x0)
    xs = [xblk(0)]
    ys = [ln1(xs[0])]
    wait(cp_wq[0])
    perm_qkv(0, rows=range(0, 16))
    for c in range(4):
        q_s[:, c * 128:(c + 1) * 128] = qhalf(0, c)
    wait(cp_wq[1])
    perm_qkv(0, rows=range(16, 32))
    wait(cp_x123)
    xs += [xblk(1), xblk(2)]
    ys += [ln1(xs[1]), ln1(xs[2]), ln1(xblk(3))]
    for c in range(4):
        ats[0].q[c] = q_s[:, c * 128:(c + 1) * 128] + qhalf(1, c)
    qt(1, [0, 1, 2, 3])
    qt(2, [0, 1, 2, 3])
    wait(cp_wk)
    perm_qkv(1)
    qt(3, [0, 1])
    qt(0, [4, 5, 6, 7])
    qt(1, [4, 5, 6, 7])
    ats[0].qk_all()
    qt(3, [2, 3])
    qt(2, [4, 5, 6, 7])
    for c in range(NC):
        ats[1].qk(c)
    qt(3, [4, 5])
    ats[1].flush()
    wait(cp_wv, cp_wo, cp_b1, cp_b2)
    perm_qkv(2)
    wo_pieces = [functools.partial(fn, cb, t) for cb in range(4) for fn in (perm_wo_a, perm_wo_b) for t in range(4)]
    for k, fn in enumerate(wo_pieces):
        tl.trigger(tl.slot + 1 + (k * 11) // 32, lambda piece, fn=fn: fn())
    l1 = lax.broadcasted_iota(jnp.int32, (1, 128), 1)
    b1_p[:, 1280:FP] = jnp.where(l1 == F - 1280, 4.0, 0.0)
    b1_p[:, 0:F] = b1_v[...].astype(f32).reshape(1, F) * 0.5
    rpad = lax.broadcasted_iota(jnp.int32, (FP - F, D), 0)
    w2_v[F:FP, :] = jnp.where(rpad == 0, b2_v[...].astype(f32).reshape(1, D) * 0.125, 0.0).astype(bf16)
    qt(3, [6, 7])
    qt(0, [8, 9, 10, 11])
    ats[0].due_at(tl.rel((3, 4, 4, 5, 6, 6, 7, 7)))
    qt(1, [8, 9, 10, 11])
    qt(2, [8, 9, 10, 11])
    halo(0, PB + P * M)
    ats[1].due_at(tl.rel((0, 1, 2, 3, 4, 5, 6, 7)))
    wblk(0)
    qt(3, [8, 9, 10, 11])
    y0 = ln2(xs[0])
    wait(cp_w1)
    ats[2].qk_all()
    ats[2].due_at(tl.rel((7, 8, 9, 10, 11, 12, 13, 14)))
    wblk(1)
    h0 = mm_M1(y0, repack=True)
    wblk(2)
    h1 = mm_M1(ln2(xs[1]))
    h2 = mm_M1(ln2(xs[2]))
    wait(cp_w2)
    x0 = mm_M2(xs[0], h0, repack=True)
    x1 = mm_M2(xs[1], h1)
    at0 = mm_Q(ln1(x0), 1, (4, 5, 6, 7, 8, 9, 10, 11), first=True, row0=PB)
    halo(1, PB + M)
    at1 = mm_Q(ln1(x1), 1, (7, 8, 9, 10, 11, 12, 13, 14))
    x0 = mm_W(x0, at0.done())
    x2 = mm_M2(xs[2], h2)
    h0 = mm_M1(ln2(x0))
    x1 = mm_W(x1, at1.done())
    halo(1, HALO + M)
    ats[3].start_at(tl.rel((0, 1, 2, 3, 4, 5, 6, 7)))
    put_out(0, mm_M2(x0, h0))
    ats[3].due_at(tl.rel(DL_LAST))
    h1 = mm_M1(ln2(x1))
    put_out(1, mm_M2(x1, h1))
    o3 = ats[3].done()
    halo(0, HALO + M)
    save(o3, x2)

    wait(cp_xr)

    def body(i, carry):
        o, x1 = load()
        for u in range(U):
            o, x1 = step(o, x1, P + i * U + u, last=(u == U - 1))
        save(o, x1)
        return carry
    lax.fori_loop(0, (NB - 1 - P) // U, body, 0)

    o, x1 = load()
    x1, x2 = step_a(o, x1, NB - 1)
    y2 = ln2(x2)
    at = mm_Q(ln1(x1), 1, DL_TAIL)
    h2 = mm_M1(y2)
    put_out(NB - 2, mm_M2(x2, h2, js=(0, 1)))
    x3 = mm_W(x1, at.done())
    put_out(NB - 2, mm_M2(x2, h2, js=(2, 3)), 256)
    h3 = mm_M1(ln2(x3))
    for j in range(4):
        put_out(NB - 1, mm_M2(x3, h3, js=(j,)), j * 128)
    cp(o_v, o_hbm, osem).wait()


@jax.jit
def pallas_interleave_layers__sliding_local_dilated__mixer_channel_mlp__prompt_kernel(
    A_x: jax.Array,
    A_wqkv: jax.Array,
    A_wo: jax.Array,
    B_x: jax.Array,
    B_w1: jax.Array,
    B_b1: jax.Array,
    B_w2: jax.Array,
    B_b2: jax.Array,
):
    assert (NB - 1 - P) % U == 0
    anyspec = pl.BlockSpec(memory_space=pl.ANY)
    out = pl.pallas_call(
        _kernel,
        in_specs=[anyspec] * 7,
        out_specs=anyspec,
        out_shape=jax.ShapeDtypeStruct((S, D), bf16),
        scratch_shapes=[
            pltpu.VMEM((S, D), bf16), pltpu.VMEM((S, D), bf16),
            pltpu.VMEM((D, 3 * D), bf16), pltpu.VMEM((D, D), bf16),
            pltpu.VMEM((F, D), bf16), pltpu.VMEM((FP, D), bf16),
            pltpu.VMEM((F,), bf16), pltpu.VMEM((D,), bf16),
            pltpu.VMEM((D // 2, 3 * D), u32), pltpu.VMEM((D // 2, D), u32),
            pltpu.VMEM((F // 2, D), u32), pltpu.VMEM((FP // 2, D), u32),
            pltpu.VMEM((1, FP), f32),
            pltpu.VMEM((4, H * WS, 128), f32),
            pltpu.VMEM((16, 4 * M + 2 * HALO, 128), f32),
            pltpu.VMEM((M // 2, D), u32), pltpu.VMEM((M, D), f32),
            pltpu.VMEM((M, D), f32),
            pltpu.VMEM((8, 128), u32),
            pltpu.SemaphoreType.DMA((12,)), pltpu.SemaphoreType.DMA(()),
        ],
        compiler_params=pltpu.CompilerParams(vmem_limit_bytes=100 << 20),
    )(A_x.reshape(S, D), A_wqkv, A_wo, B_w1.T, B_b1, B_w2, B_b2)
    return out.reshape(1, S, D)
```

```python
import functools
import math

import jax
import jax.numpy as jnp
import numpy as np
from jax import lax
import jax.experimental.pallas as pl
import jax.experimental.pallas.tpu as pltpu

S, D, F = 2048, 512, 1376
FP = 1408
H, DH, W, DIL = 32, 16, 8, 2
HALO = 16
WS = 20
EPS = 1e-5
LOG2E = 1.4426950408889634
QSCALE = (DH ** -0.5) * LOG2E
QSCALE_BITS = int(np.float32(QSCALE).view(np.uint32))
NEG = -1e9 * LOG2E
f32, bf16, u32 = jnp.float32, jnp.bfloat16, jnp.uint32

M = 128
NB = S // M
RC = 16
RA = 16
NC = M // RA
P = 3
U = 2
PB = 2 * HALO + M

NB_SLOTS = (-5, -4, -3, -2, -1, 0, 1, 2)
DL_SLOTS = (15, 16, 17, 18, 19, 20, 21, 22)
DL_LAST = (14, 15, 16, 17, 18, 19, 20, 21)
DL_TAIL = (8, 9, 10, 12, 13, 14, 15, 16)
M1_ORDER = (0, 1, 2, 3, 10, 4, 5, 6, 7, 8, 9)


def _ln(x):
    m = jnp.mean(x, axis=-1, keepdims=True)
    xc = x - m
    v = jnp.mean(xc * xc, axis=-1, keepdims=True)
    return xc * lax.rsqrt(v + EPS)


def _ln_half(x):
    m = jnp.mean(x, axis=-1, keepdims=True)
    xc = x - m
    v4 = jnp.sum(xc * xc, axis=-1, keepdims=True) * (4.0 / D)
    return xc * lax.rsqrt(v4 + 4.0 * EPS)


def _gelu_from_half(z):
    c = math.sqrt(2.0 / math.pi)
    inner = z * (2.0 * c + (8.0 * c * 0.044715) * (z * z))
    return z + z * jnp.tanh(inner)


def _dot(a, b):
    return jnp.dot(a, b, preferred_element_type=f32)


def _dot_t(a, b):
    return lax.dot_general(a, b, (((1,), (1,)), ((), ())), preferred_element_type=f32)


def _or_all(xs):
    return functools.reduce(lambda u, v: u | v, xs)


def _pieces(a):
    return [a[r:r + 8, c:c + 128] for r in range(0, a.shape[0], 8) for c in range(0, a.shape[1], 128)]


def _patch(wu, r, tok):
    rows = wu[r:r + 8]
    if wu.shape[1] > 128:
        rows = jnp.concatenate([rows[:, 0:128] | tok, rows[:, 128:]], axis=1)
    else:
        rows = rows | tok
    parts = ([wu[:r]] if r > 0 else []) + [rows] + ([wu[r + 8:]] if r + 8 < wu.shape[0] else [])
    return jnp.concatenate(parts, axis=0)


class _Timeline:
    def __init__(self):
        self.slot, self.due, self.trig = 0, {}, {}

    def rel(self, offs):
        return [self.slot + o for o in offs]

    def deadline(self, slot, fn):
        self.due.setdefault(slot, []).append(fn)

    def trigger(self, slot, fn):
        self.trig.setdefault(slot, []).append(fn)

    def weights(self, wu, r=0, off=0):
        for fn in self.due.pop(self.slot + off, []):
            wu = _patch(wu, r, fn())
        return wu

    def done(self, r, n=1):
        lo = self.slot
        self.slot += n
        for s in range(lo, self.slot):
            for fn in self.trig.pop(s, []):
                fn(r[r.shape[0] - 8:, 0:128])

    def barrier(self):
        assert not self.trig
        self.due.clear()


def _kernel(x_hbm, wqkv_hbm, wo_hbm, w1t_hbm, b1_hbm, w2_hbm, b2_hbm, o_hbm,
            x_v, o_v, wqkv_v, wo_v, w1_v, w2_v, b1_v, b2_v,
            wqkv_p, wo_p, w1_p, w2_p, b1_p, wo_tmp, kv, o_s, q_s, x1_s, zero_s, sems, osem):
    tl = _Timeline()

    XE = (P + 1) * M
    cp = pltpu.make_async_copy
    cp_x0 = cp(x_hbm.at[0:M], x_v.at[0:M], sems.at[0])
    cp_wq = [cp(wqkv_hbm.at[hf * 256:(hf + 1) * 256, 0:D], wqkv_v.at[hf * 256:(hf + 1) * 256, 0:D], sems.at[1 + hf])
             for hf in range(2)]
    cp_x123 = cp(x_hbm.at[M:XE], x_v.at[M:XE], sems.at[3])
    cp_wk = cp(wqkv_hbm.at[:, D:2 * D], wqkv_v.at[:, D:2 * D], sems.at[4])
    cp_wv = cp(wqkv_hbm.at[:, 2 * D:3 * D], wqkv_v.at[:, 2 * D:3 * D], sems.at[5])
    cp_wo = cp(wo_hbm, wo_v, sems.at[6])
    cp_b1 = cp(b1_hbm, b1_v, sems.at[7])
    cp_b2 = cp(b2_hbm, b2_v, sems.at[8])
    cp_w1 = cp(w1t_hbm, w1_v, sems.at[9])
    cp_w2 = cp(w2_hbm, w2_v.at[0:F], sems.at[10])
    cp_xr = cp(x_hbm.at[XE:S], x_v.at[XE:S], sems.at[11])
    for c_ in [cp_x0, cp_wq[0], cp_wq[1], cp_x123, cp_wk, cp_wv, cp_wo, cp_b1, cp_b2, cp_w1, cp_w2, cp_xr]:
        c_.start()

    def wait(*cps):
        tl.barrier()
        for c_ in cps:
            c_.wait()

    def rowslice(n):
        r = n * M
        if not isinstance(n, int):
            r = pl.multiple_of(r, M)
        return pl.ds(r, M)

    lane = lax.broadcasted_iota(jnp.int32, (8, 128), 1)
    dq = (lane % 16) // 4
    g_, j_, h_ = lane // 32, (lane % 32) // 8, lane % 8
    idx = [h_ * 16 + 4 * ((i + j_) % 4) + g_ for i in range(4)]
    msk = [dq == t for t in range(4)]

    def perm_qkv(t, rows=range(D // 16)):
        for i in range(4):
            for r in rows:
                src = [pltpu.bitcast(wqkv_v[r * 16:(r + 1) * 16, t * D + j * 128: t * D + (j + 1) * 128], u32)
                       for j in range(4)]
                m = src[(0 - i) % 4]
                for tq in range(1, 4):
                    m = jnp.where(msk[tq], src[(tq - i) % 4], m)
                wqkv_p[r * 8:(r + 1) * 8, t * D + i * 128: t * D + (i + 1) * 128] = \
                    jnp.take_along_axis(m, idx[i], axis=1)

    def perm_wo_a(cb, j):
        for hh in range(8 * j, 8 * j + 8):
            wo_tmp[cb, hh * WS:hh * WS + DH, :] = wo_v[hh * DH:(hh + 1) * DH, cb * 128:(cb + 1) * 128].astype(f32)

    def perm_wo_b(cb, i):
        for g in range(4):
            rows = [wo_tmp[cb, pl.ds(j * 8 * WS + 4 * ((i + j) % 4) + g, 8, stride=WS), :] for j in range(4)]
            r0 = (i * 128 + g * 32) // 2
            wo_p[r0:r0 + 16, cb * 128:(cb + 1) * 128] = \
                pltpu.bitcast(jnp.concatenate(rows, axis=0).astype(bf16), u32)

    def ztok(pieces):
        return _or_all([pltpu.bitcast(p, u32) for p in pieces]) & zero_s[...]

    def rows_map(fn, x):
        return jnp.concatenate([fn(x[r:r + RC]) for r in range(0, x.shape[0], RC)], axis=0)

    def ln1(x):
        return rows_map(_ln, x).astype(bf16)

    def ln2(x):
        return rows_map(lambda a: _ln_half(_ln(a)), x).astype(bf16)

    def halo(layer, end):
        L = layer * 8
        kv[L:L + 8, 0:HALO, :] = kv[L:L + 8, end - HALO:end, :]

    class Attn:
        def __init__(self, layer, first=False, row0=HALO):
            self.layer, self.first, self.row0 = layer, first, row0
            self.q = [None] * 4
            self.half, self.logit, self.outs = {}, {}, {}

        def qk(self, c, tok=None):
            L, r0 = self.layer * 8, c * RA
            g0 = self.row0 + r0
            if tok is None:
                sc = QSCALE
            else:
                sc = jnp.concatenate([pltpu.bitcast(tok | QSCALE_BITS, f32)] * (RA // 8), axis=0)
            qs = [self.q[j][r0:r0 + RA] * sc for j in range(4)]
            ls = []
            for w in range(W):
                s = None
                for j in range(4):
                    t = qs[j] * kv[L + j, pl.ds(g0 - DIL * w, RA), :]
                    s = t if s is None else s + t
                ls.append(s)
            self.half[c] = [s + pltpu.roll(s, 64, 1) for s in ls]
            for c2 in sorted(self.half):
                if c2 < c:
                    self.qkb(c2)

        def qkb(self, c):
            r0 = c * RA
            ls = [s + pltpu.roll(s, 32, 1) for s in self.half.pop(c)]
            if self.first and r0 < HALO:
                row = r0 + lax.broadcasted_iota(jnp.int32, (RA, 128), 0)
                ls = [ls[0]] + [jnp.where(row >= DIL * w, ls[w], NEG) for w in range(1, W)]
            self.logit[c] = ls

        def flush(self):
            for c in sorted(self.half):
                self.qkb(c)

        def qk_all(self):
            for c in range(NC):
                self.qk(c)
            self.flush()

        def av(self, c):
            L, r0 = self.layer * 8, c * RA
            g0 = self.row0 + r0
            ls = self.logit[c]
            m = ls[0]
            for w in range(1, W):
                m = jnp.maximum(m, ls[w])
            ps = [jnp.exp2(l - m) for l in ls]
            den = ps[0]
            for w in range(1, W):
                den = den + ps[w]
            inv = pl.reciprocal(den, approx=True)
            inv = inv * (2.0 - den * inv)
            oj = []
            for j in range(4):
                a = None
                for w in range(W):
                    t = ps[w] * kv[L + 4 + j, pl.ds(g0 - DIL * w, RA), :]
                    a = t if a is None else a + t
                oj.append(a * inv)
            self.outs[c] = jnp.concatenate(oj, axis=1)

        def finish(self, c):
            assert c in self.logit or c in self.half
            if c in self.half:
                self.qkb(c)
            if c not in self.outs:
                self.av(c)

        def start_at(self, slots):
            for c, s in enumerate(slots):
                tl.trigger(s, lambda piece, c=c: self.qk(c, ztok([piece])))

        def due_at(self, slots):
            def tok(c):
                self.finish(c)
                return ztok(_pieces(self.outs[c]))
            for c, s in enumerate(slots):
                tl.deadline(s, lambda c=c: tok(c))

        def done(self):
            for c in range(NC):
                self.finish(c)
            return jnp.concatenate([self.outs[c] for c in range(NC)], axis=0).astype(bf16)

    def q_tile(at, y, c):
        wu = tl.weights(wqkv_p[:, c * 128:(c + 1) * 128])
        r = _dot(y, pltpu.bitcast(wu, bf16))
        if c < 4:
            at.q[c] = r
        else:
            kv[at.layer * 8 + c - 4, at.row0:at.row0 + M, :] = r
        tl.done(r)

    def mm_Q(y, layer, dl, first=False, row0=HALO):
        at = Attn(layer, first=first, row0=row0)
        end = tl.slot + 12
        at.start_at([end + s for s in NB_SLOTS])
        at.due_at([end + s for s in dl])
        for c in range(12):
            q_tile(at, y, c)
        return at

    def mm_W(x, o):
        outs = []
        for j in range(4):
            cs = slice(j * 128, (j + 1) * 128)
            r = _dot(o, pltpu.bitcast(tl.weights(wo_p[:, cs]), bf16))
            tl.done(r)
            outs.append(x[:, cs] + r)
        return jnp.concatenate(outs, axis=1)

    def mm_M1(y, repack=False):
        hs = {}
        for t in M1_ORDER:
            n0 = t * 128
            nr = min(128, F - n0)
            if repack:
                wu = pltpu.bitcast(w1_v[n0:n0 + nr, :], u32)
                w1_p[n0 // 2:(n0 + nr) // 2, :] = wu
            else:
                wu = w1_p[n0 // 2:(n0 + nr) // 2, :]
            w = pltpu.bitcast(tl.weights(wu), bf16)
            if nr == 128:
                r = _dot_t(y, w)
                tl.done(r)
            else:
                rt = _dot_t(w, y)
                tl.done(rt)
                r = jnp.concatenate([rt, jnp.zeros((128 - nr, M), f32)], axis=0).T
            hs[t] = _gelu_from_half(r + b1_p[:, n0:n0 + 128])
        return jnp.concatenate([hs[t] for t in range(FP // 128)], axis=1).astype(bf16)

    def mm_M2(x, h, repack=False, js=(0, 1, 2, 3)):
        outs = []
        for j in js:
            cs = slice(j * 128, (j + 1) * 128)
            if repack:
                wu = pltpu.bitcast(w2_v[:, cs], u32)
                w2_p[:, cs] = wu
            else:
                wu = w2_p[:, cs]
            ps = [p for p in range(11) if (4 * p) // 11 == j]
            for i, p in enumerate(ps):
                wu = tl.weights(wu, ((4 * p) % 11) * 64, off=i)
            r = _dot(h, pltpu.bitcast(wu, bf16))
            tl.done(r, len(ps))
            outs.append(x[:, cs] + r)
        return jnp.concatenate(outs, axis=1)

    def xblk(n):
        return x_v[rowslice(n), :].astype(f32)

    def put_out(n, val, c0=0):
        cs = slice(c0, c0 + val.shape[1])
        o_v[rowslice(n), cs] = val.astype(bf16)
        cp(o_v.at[rowslice(n), cs], o_hbm.at[rowslice(n), cs], osem).start()

    def save(o, x1):
        x1_s[...] = x1
        o_s[...] = pltpu.bitcast(o, u32)
        tl.barrier()

    def load():
        return pltpu.bitcast(o_s[...], bf16), x1_s[...]

    def step_a(o, x1, n):
        x = mm_W(xblk(n), o)
        y = ln2(x)
        at = mm_Q(ln1(x1), 1, DL_SLOTS)
        h = mm_M1(y)
        x1n = mm_M2(x, h)
        x2 = mm_W(x1, at.done())
        halo(1, HALO + M)
        return x1n, x2

    def step(o, x1, n, last):
        x1n, x2 = step_a(o, x1, n)
        y2 = ln2(x2)
        at = mm_Q(ln1(xblk(n + 1)), 0, DL_LAST if last else DL_SLOTS)
        h2 = mm_M1(y2)
        put_out(n - 1, mm_M2(x2, h2))
        on = at.done()
        halo(0, HALO + M)
        return on, x1n

    kv[:, PB - HALO:PB, :] = jnp.zeros((16, HALO, 128), f32)
    zero_s[...] = jnp.zeros((8, 128), u32)
    ats = [Attn(0, first=(b == 0), row0=PB + b * M) for b in range(P)] + [Attn(0)]

    def qt(b, cs):
        for c in cs:
            q_tile(ats[b], ys[b], c)

    def wblk(b):
        xs[b] = mm_W(xs[b], ats[b].done())

    def qhalf(hf, c):
        w = pltpu.bitcast(wqkv_p[hf * 128:(hf + 1) * 128, c * 128:(c + 1) * 128], bf16)
        return _dot(ys[0][:, hf * 256:(hf + 1) * 256], w)

    wait(cp_x0)
    xs = [xblk(0)]
    ys = [ln1(xs[0])]
    wait(cp_wq[0])
    perm_qkv(0, rows=range(0, 16))
    for c in range(4):
        q_s[:, c * 128:(c + 1) * 128] = qhalf(0, c)
    wait(cp_wq[1])
    perm_qkv(0, rows=range(16, 32))
    wait(cp_x123)
    xs += [xblk(1), xblk(2)]
    ys += [ln1(xs[1]), ln1(xs[2]), ln1(xblk(3))]
    for c in range(4):
        ats[0].q[c] = q_s[:, c * 128:(c + 1) * 128] + qhalf(1, c)
    qt(1, [0, 1, 2, 3])
    qt(2, [0, 1, 2, 3])
    wait(cp_wk)
    perm_qkv(1)
    qt(3, [0, 1])
    qt(0, [4, 5, 6, 7])
    qt(1, [4, 5, 6, 7])
    ats[0].qk_all()
    qt(3, [2, 3])
    qt(2, [4, 5, 6, 7])
    for c in range(NC):
        ats[1].qk(c)
    qt(3, [4, 5])
    ats[1].flush()
    wait(cp_wv, cp_wo, cp_b1, cp_b2)
    perm_qkv(2)
    wo_pieces = [functools.partial(fn, cb, t) for cb in range(4) for fn in (perm_wo_a, perm_wo_b) for t in range(4)]
    for k, fn in enumerate(wo_pieces):
        tl.trigger(tl.slot + 1 + (k * 11) // 32, lambda piece, fn=fn: fn())
    l1 = lax.broadcasted_iota(jnp.int32, (1, 128), 1)
    b1_p[:, 1280:FP] = jnp.where(l1 == F - 1280, 4.0, 0.0)
    b1_p[:, 0:F] = b1_v[...].astype(f32).reshape(1, F) * 0.5
    rpad = lax.broadcasted_iota(jnp.int32, (FP - F, D), 0)
    w2_v[F:FP, :] = jnp.where(rpad == 0, b2_v[...].astype(f32).reshape(1, D) * 0.125, 0.0).astype(bf16)
    qt(3, [6, 7])
    qt(0, [8, 9, 10, 11])
    ats[0].due_at(tl.rel((3, 4, 4, 5, 6, 6, 7, 7)))
    qt(1, [8, 9, 10, 11])
    qt(2, [8, 9, 10, 11])
    halo(0, PB + P * M)
    ats[1].due_at(tl.rel((0, 1, 2, 3, 4, 5, 6, 7)))
    wblk(0)
    qt(3, [8, 9, 10, 11])
    y0 = ln2(xs[0])
    wait(cp_w1)
    ats[2].qk_all()
    ats[2].due_at(tl.rel((6, 7, 8, 9, 10, 11, 12, 13)))
    wblk(1)
    h0 = mm_M1(y0, repack=True)
    wblk(2)
    h1 = mm_M1(ln2(xs[1]))
    h2 = mm_M1(ln2(xs[2]))
    wait(cp_w2)
    x0 = mm_M2(xs[0], h0, repack=True)
    x1 = mm_M2(xs[1], h1)
    at0 = mm_Q(ln1(x0), 1, (5, 6, 7, 8, 9, 10, 11, 12), first=True, row0=PB)
    halo(1, PB + M)
    at1 = mm_Q(ln1(x1), 1, (10, 12, 14, 16, 18, 20, 22, 24))
    x0 = mm_W(x0, at0.done())
    x2 = mm_M2(xs[2], h2)
    h0 = mm_M1(ln2(x0))
    x1 = mm_W(x1, at1.done())
    halo(1, HALO + M)
    ats[3].start_at(tl.rel((0, 1, 2, 3, 4, 5, 6, 7)))
    put_out(0, mm_M2(x0, h0))
    ats[3].due_at(tl.rel(DL_LAST))
    h1 = mm_M1(ln2(x1))
    put_out(1, mm_M2(x1, h1))
    o3 = ats[3].done()
    halo(0, HALO + M)
    save(o3, x2)

    wait(cp_xr)

    def body(i, carry):
        o, x1 = load()
        for u in range(U):
            o, x1 = step(o, x1, P + i * U + u, last=(u == U - 1))
        save(o, x1)
        return carry
    lax.fori_loop(0, (NB - 1 - P) // U, body, 0)

    o, x1 = load()
    x1, x2 = step_a(o, x1, NB - 1)
    y2 = ln2(x2)
    at = mm_Q(ln1(x1), 1, DL_TAIL)
    h2 = mm_M1(y2)
    put_out(NB - 2, mm_M2(x2, h2, js=(0, 1)))
    x3 = mm_W(x1, at.done())
    put_out(NB - 2, mm_M2(x2, h2, js=(2, 3)), 256)
    h3 = mm_M1(ln2(x3))
    for j in range(4):
        put_out(NB - 1, mm_M2(x3, h3, js=(j,)), j * 128)
    cp(o_v, o_hbm, osem).wait()


@jax.jit
def pallas_interleave_layers__sliding_local_dilated__mixer_channel_mlp__prompt_kernel(
    A_x: jax.Array,
    A_wqkv: jax.Array,
    A_wo: jax.Array,
    B_x: jax.Array,
    B_w1: jax.Array,
    B_b1: jax.Array,
    B_w2: jax.Array,
    B_b2: jax.Array,
):
    assert (NB - 1 - P) % U == 0
    anyspec = pl.BlockSpec(memory_space=pl.ANY)
    out = pl.pallas_call(
        _kernel,
        in_specs=[anyspec] * 7,
        out_specs=anyspec,
        out_shape=jax.ShapeDtypeStruct((S, D), bf16),
        scratch_shapes=[
            pltpu.VMEM((S, D), bf16), pltpu.VMEM((S, D), bf16),
            pltpu.VMEM((D, 3 * D), bf16), pltpu.VMEM((D, D), bf16),
            pltpu.VMEM((F, D), bf16), pltpu.VMEM((FP, D), bf16),
            pltpu.VMEM((F,), bf16), pltpu.VMEM((D,), bf16),
            pltpu.VMEM((D // 2, 3 * D), u32), pltpu.VMEM((D // 2, D), u32),
            pltpu.VMEM((F // 2, D), u32), pltpu.VMEM((FP // 2, D), u32),
            pltpu.VMEM((1, FP), f32),
            pltpu.VMEM((4, H * WS, 128), f32),
            pltpu.VMEM((16, 4 * M + 2 * HALO, 128), f32),
            pltpu.VMEM((M // 2, D), u32), pltpu.VMEM((M, D), f32),
            pltpu.VMEM((M, D), f32),
            pltpu.VMEM((8, 128), u32),
            pltpu.SemaphoreType.DMA((12,)), pltpu.SemaphoreType.DMA(()),
        ],
        compiler_params=pltpu.CompilerParams(vmem_limit_bytes=100 << 20),
    )(A_x.reshape(S, D), A_wqkv, A_wo, B_w1.T, B_b1, B_w2, B_b2)
    return out.reshape(1, S, D)
```

```python
import functools
import math

import jax
import jax.numpy as jnp
import numpy as np
from jax import lax
import jax.experimental.pallas as pl
import jax.experimental.pallas.tpu as pltpu

S, D, F = 2048, 512, 1376
FP = 1408
H, DH, W, DIL = 32, 16, 8, 2
HALO = 16
WS = 20
EPS = 1e-5
LOG2E = 1.4426950408889634
QSCALE = (DH ** -0.5) * LOG2E
QSCALE_BITS = int(np.float32(QSCALE).view(np.uint32))
NEG = -1e9 * LOG2E
f32, bf16, u32 = jnp.float32, jnp.bfloat16, jnp.uint32

M = 128
NB = S // M
RC = 16
RA = 16
NC = M // RA
P = 3
U = 2
PB = 2 * HALO + M

NB_SLOTS = (-5, -4, -3, -2, -1, 0, 1, 2)
DL_SLOTS = (15, 16, 17, 18, 19, 20, 21, 22)
DL_LAST = (14, 15, 16, 17, 18, 19, 20, 21)
DL_TAIL = (8, 9, 10, 12, 13, 14, 15, 16)
M1_ORDER = (0, 1, 2, 3, 10, 4, 5, 6, 7, 8, 9)


def _ln(x):
    m = jnp.mean(x, axis=-1, keepdims=True)
    xc = x - m
    v = jnp.mean(xc * xc, axis=-1, keepdims=True)
    return xc * lax.rsqrt(v + EPS)


def _ln_half(x):
    m = jnp.mean(x, axis=-1, keepdims=True)
    xc = x - m
    v4 = jnp.sum(xc * xc, axis=-1, keepdims=True) * (4.0 / D)
    return xc * lax.rsqrt(v4 + 4.0 * EPS)


def _gelu_from_half(z):
    c = math.sqrt(2.0 / math.pi)
    inner = z * (2.0 * c + (8.0 * c * 0.044715) * (z * z))
    return z + z * jnp.tanh(inner)


def _dot(a, b):
    return jnp.dot(a, b, preferred_element_type=f32)


def _dot_t(a, b):
    return lax.dot_general(a, b, (((1,), (1,)), ((), ())), preferred_element_type=f32)


def _or_all(xs):
    return functools.reduce(lambda u, v: u | v, xs)


def _pieces(a):
    return [a[r:r + 8, c:c + 128] for r in range(0, a.shape[0], 8) for c in range(0, a.shape[1], 128)]


def _patch(wu, r, tok):
    rows = wu[r:r + 8]
    if wu.shape[1] > 128:
        rows = jnp.concatenate([rows[:, 0:128] | tok, rows[:, 128:]], axis=1)
    else:
        rows = rows | tok
    parts = ([wu[:r]] if r > 0 else []) + [rows] + ([wu[r + 8:]] if r + 8 < wu.shape[0] else [])
    return jnp.concatenate(parts, axis=0)


class _Timeline:
    def __init__(self):
        self.slot, self.due, self.trig = 0, {}, {}

    def rel(self, offs):
        return [self.slot + o for o in offs]

    def deadline(self, slot, fn):
        self.due.setdefault(slot, []).append(fn)

    def trigger(self, slot, fn):
        self.trig.setdefault(slot, []).append(fn)

    def weights(self, wu, r=0, off=0):
        for fn in self.due.pop(self.slot + off, []):
            wu = _patch(wu, r, fn())
        return wu

    def done(self, r, n=1):
        lo = self.slot
        self.slot += n
        for s in range(lo, self.slot):
            for fn in self.trig.pop(s, []):
                fn(r[r.shape[0] - 8:, 0:128])

    def barrier(self):
        assert not self.trig
        self.due.clear()


def _kernel(x_hbm, wqkv_hbm, wo_hbm, w1t_hbm, b1_hbm, w2_hbm, b2_hbm, o_hbm,
            x_v, o_v, wqkv_v, wo_v, w1_v, w2_v, b1_v, b2_v,
            wqkv_p, wo_p, w1_p, w2_p, b1_p, wo_tmp, kv, o_s, q_s, x1_s, zero_s, sems, osem):
    tl = _Timeline()

    XE = (P + 1) * M
    cp = pltpu.make_async_copy
    cp_x0 = cp(x_hbm.at[0:M], x_v.at[0:M], sems.at[0])
    cp_wq = [cp(wqkv_hbm.at[hf * 256:(hf + 1) * 256, 0:D], wqkv_v.at[hf * 256:(hf + 1) * 256, 0:D], sems.at[1 + hf])
             for hf in range(2)]
    cp_x123 = cp(x_hbm.at[M:XE], x_v.at[M:XE], sems.at[3])
    cp_wk = cp(wqkv_hbm.at[:, D:2 * D], wqkv_v.at[:, D:2 * D], sems.at[4])
    cp_wv = cp(wqkv_hbm.at[:, 2 * D:3 * D], wqkv_v.at[:, 2 * D:3 * D], sems.at[5])
    cp_wo = cp(wo_hbm, wo_v, sems.at[6])
    cp_b1 = cp(b1_hbm, b1_v, sems.at[7])
    cp_b2 = cp(b2_hbm, b2_v, sems.at[8])
    cp_w1 = cp(w1t_hbm, w1_v, sems.at[9])
    cp_w2 = cp(w2_hbm, w2_v.at[0:F], sems.at[10])
    cp_xr = cp(x_hbm.at[XE:S], x_v.at[XE:S], sems.at[11])
    for c_ in [cp_x0, cp_wq[0], cp_wq[1], cp_x123, cp_wk, cp_wv, cp_wo, cp_b1, cp_b2, cp_w1, cp_w2, cp_xr]:
        c_.start()

    def wait(*cps):
        tl.barrier()
        for c_ in cps:
            c_.wait()

    def rowslice(n):
        r = n * M
        if not isinstance(n, int):
            r = pl.multiple_of(r, M)
        return pl.ds(r, M)

    lane = lax.broadcasted_iota(jnp.int32, (8, 128), 1)
    dq = (lane % 16) // 4
    g_, j_, h_ = lane // 32, (lane % 32) // 8, lane % 8
    idx = [h_ * 16 + 4 * ((i + j_) % 4) + g_ for i in range(4)]
    msk = [dq == t for t in range(4)]

    def perm_qkv(t, rows=range(D // 16)):
        for i in range(4):
            for r in rows:
                src = [pltpu.bitcast(wqkv_v[r * 16:(r + 1) * 16, t * D + j * 128: t * D + (j + 1) * 128], u32)
                       for j in range(4)]
                m = src[(0 - i) % 4]
                for tq in range(1, 4):
                    m = jnp.where(msk[tq], src[(tq - i) % 4], m)
                wqkv_p[r * 8:(r + 1) * 8, t * D + i * 128: t * D + (i + 1) * 128] = \
                    jnp.take_along_axis(m, idx[i], axis=1)

    wo_outs = [[] for _ in range(4)]

    def perm_wo_a(cb, j):
        for hh in range(8 * j, 8 * j + 8):
            wo_tmp[cb, hh * WS:hh * WS + DH, :] = wo_v[hh * DH:(hh + 1) * DH, cb * 128:(cb + 1) * 128].astype(f32)

    def perm_wo_b(cb, i):
        for g in range(4):
            rows = [wo_tmp[cb, pl.ds(j * 8 * WS + 4 * ((i + j) % 4) + g, 8, stride=WS), :] for j in range(4)]
            blk = pltpu.bitcast(jnp.concatenate(rows, axis=0).astype(bf16), u32)
            r0 = (i * 128 + g * 32) // 2
            wo_p[r0:r0 + 16, cb * 128:(cb + 1) * 128] = blk
            wo_outs[cb] += [blk[0:8], blk[8:16]]

    def ztok(pieces):
        return _or_all([pltpu.bitcast(p, u32) for p in pieces]) & zero_s[...]

    def rows_map(fn, x):
        return jnp.concatenate([fn(x[r:r + RC]) for r in range(0, x.shape[0], RC)], axis=0)

    def ln1(x):
        return rows_map(_ln, x).astype(bf16)

    def ln2(x):
        return rows_map(lambda a: _ln_half(_ln(a)), x).astype(bf16)

    def halo(layer, end):
        L = layer * 8
        kv[L:L + 8, 0:HALO, :] = kv[L:L + 8, end - HALO:end, :]

    class Attn:
        def __init__(self, layer, first=False, row0=HALO):
            self.layer, self.first, self.row0 = layer, first, row0
            self.q = [None] * 4
            self.half, self.logit, self.outs = {}, {}, {}

        def qk(self, c, tok=None):
            L, r0 = self.layer * 8, c * RA
            g0 = self.row0 + r0
            if tok is None:
                sc = QSCALE
            else:
                sc = jnp.concatenate([pltpu.bitcast(tok | QSCALE_BITS, f32)] * (RA // 8), axis=0)
            qs = [self.q[j][r0:r0 + RA] * sc for j in range(4)]
            ls = []
            for w in range(W):
                s = None
                for j in range(4):
                    t = qs[j] * kv[L + j, pl.ds(g0 - DIL * w, RA), :]
                    s = t if s is None else s + t
                ls.append(s)
            self.half[c] = [s + pltpu.roll(s, 64, 1) for s in ls]
            for c2 in sorted(self.half):
                if c2 < c:
                    self.qkb(c2)

        def qkb(self, c):
            r0 = c * RA
            ls = [s + pltpu.roll(s, 32, 1) for s in self.half.pop(c)]
            if self.first and r0 < HALO:
                row = r0 + lax.broadcasted_iota(jnp.int32, (RA, 128), 0)
                ls = [ls[0]] + [jnp.where(row >= DIL * w, ls[w], NEG) for w in range(1, W)]
            self.logit[c] = ls

        def flush(self):
            for c in sorted(self.half):
                self.qkb(c)

        def qk_all(self):
            for c in range(NC):
                self.qk(c)
            self.flush()

        def av(self, c):
            L, r0 = self.layer * 8, c * RA
            g0 = self.row0 + r0
            ls = self.logit[c]
            m = ls[0]
            for w in range(1, W):
                m = jnp.maximum(m, ls[w])
            ps = [jnp.exp2(l - m) for l in ls]
            den = ps[0]
            for w in range(1, W):
                den = den + ps[w]
            inv = pl.reciprocal(den, approx=True)
            inv = inv * (2.0 - den * inv)
            oj = []
            for j in range(4):
                a = None
                for w in range(W):
                    t = ps[w] * kv[L + 4 + j, pl.ds(g0 - DIL * w, RA), :]
                    a = t if a is None else a + t
                oj.append(a * inv)
            self.outs[c] = jnp.concatenate(oj, axis=1)

        def finish(self, c):
            assert c in self.logit or c in self.half
            if c in self.half:
                self.qkb(c)
            if c not in self.outs:
                self.av(c)

        def start_at(self, slots):
            for c, s in enumerate(slots):
                tl.trigger(s, lambda piece, c=c: self.qk(c, ztok([piece])))

        def due_at(self, slots):
            def tok(c):
                self.finish(c)
                return ztok(_pieces(self.outs[c]))
            for c, s in enumerate(slots):
                tl.deadline(s, lambda c=c: tok(c))

        def done(self):
            for c in range(NC):
                self.finish(c)
            return jnp.concatenate([self.outs[c] for c in range(NC)], axis=0).astype(bf16)

    def q_tile(at, y, c):
        wu = tl.weights(wqkv_p[:, c * 128:(c + 1) * 128])
        r = _dot(y, pltpu.bitcast(wu, bf16))
        if c < 4:
            at.q[c] = r
        else:
            kv[at.layer * 8 + c - 4, at.row0:at.row0 + M, :] = r
        tl.done(r)

    def mm_Q(y, layer, dl, first=False, row0=HALO):
        at = Attn(layer, first=first, row0=row0)
        end = tl.slot + 12
        at.start_at([end + s for s in NB_SLOTS])
        at.due_at([end + s for s in dl])
        for c in range(12):
            q_tile(at, y, c)
        return at

    def mm_W(x, o):
        outs = []
        for j in range(4):
            cs = slice(j * 128, (j + 1) * 128)
            r = _dot(o, pltpu.bitcast(tl.weights(wo_p[:, cs]), bf16))
            tl.done(r)
            outs.append(x[:, cs] + r)
        return jnp.concatenate(outs, axis=1)

    def mm_M1(y, repack=False):
        hs = {}
        for t in M1_ORDER:
            n0 = t * 128
            nr = min(128, F - n0)
            if repack:
                wu = pltpu.bitcast(w1_v[n0:n0 + nr, :], u32)
                w1_p[n0 // 2:(n0 + nr) // 2, :] = wu
            else:
                wu = w1_p[n0 // 2:(n0 + nr) // 2, :]
            w = pltpu.bitcast(tl.weights(wu), bf16)
            if nr == 128:
                r = _dot_t(y, w)
                tl.done(r)
            else:
                rt = _dot_t(w, y)
                tl.done(rt)
                r = jnp.concatenate([rt, jnp.zeros((128 - nr, M), f32)], axis=0).T
            hs[t] = _gelu_from_half(r + b1_p[:, n0:n0 + 128])
        return jnp.concatenate([hs[t] for t in range(FP // 128)], axis=1).astype(bf16)

    def mm_M2(x, h, repack=False, js=(0, 1, 2, 3)):
        outs = []
        for j in js:
            cs = slice(j * 128, (j + 1) * 128)
            if repack:
                wu = pltpu.bitcast(w2_v[:, cs], u32)
                w2_p[:, cs] = wu
            else:
                wu = w2_p[:, cs]
            ps = [p for p in range(11) if (4 * p) // 11 == j]
            for i, p in enumerate(ps):
                wu = tl.weights(wu, ((4 * p) % 11) * 64, off=i)
            r = _dot(h, pltpu.bitcast(wu, bf16))
            tl.done(r, len(ps))
            outs.append(x[:, cs] + r)
        return jnp.concatenate(outs, axis=1)

    def xblk(n):
        return x_v[rowslice(n), :].astype(f32)

    def put_out(n, val, c0=0):
        cs = slice(c0, c0 + val.shape[1])
        o_v[rowslice(n), cs] = val.astype(bf16)
        cp(o_v.at[rowslice(n), cs], o_hbm.at[rowslice(n), cs], osem).start()

    def save(o, x1):
        x1_s[...] = x1
        o_s[...] = pltpu.bitcast(o, u32)
        tl.barrier()

    def load():
        return pltpu.bitcast(o_s[...], bf16), x1_s[...]

    def step_a(o, x1, n):
        x = mm_W(xblk(n), o)
        y = ln2(x)
        at = mm_Q(ln1(x1), 1, DL_SLOTS)
        h = mm_M1(y)
        x1n = mm_M2(x, h)
        x2 = mm_W(x1, at.done())
        halo(1, HALO + M)
        return x1n, x2

    def step(o, x1, n, last):
        x1n, x2 = step_a(o, x1, n)
        y2 = ln2(x2)
        at = mm_Q(ln1(xblk(n + 1)), 0, DL_LAST if last else DL_SLOTS)
        h2 = mm_M1(y2)
        put_out(n - 1, mm_M2(x2, h2))
        on = at.done()
        halo(0, HALO + M)
        return on, x1n

    kv[:, PB - HALO:PB, :] = jnp.zeros((16, HALO, 128), f32)
    zero_s[...] = jnp.zeros((8, 128), u32)
    ats = [Attn(0, first=(b == 0), row0=PB + b * M) for b in range(P)] + [Attn(0)]

    def qt(b, cs):
        for c in cs:
            q_tile(ats[b], ys[b], c)

    def wblk(b):
        xs[b] = mm_W(xs[b], ats[b].done())

    def qhalf(hf, c):
        w = pltpu.bitcast(wqkv_p[hf * 128:(hf + 1) * 128, c * 128:(c + 1) * 128], bf16)
        return _dot(ys[0][:, hf * 256:(hf + 1) * 256], w)

    wait(cp_x0)
    xs = [xblk(0)]
    ys = [ln1(xs[0])]
    wait(cp_wq[0])
    perm_qkv(0, rows=range(0, 16))
    for c in range(4):
        q_s[:, c * 128:(c + 1) * 128] = qhalf(0, c)
    wait(cp_wq[1])
    perm_qkv(0, rows=range(16, 32))
    wait(cp_x123)
    xs += [xblk(1), xblk(2)]
    ys += [ln1(xs[1]), ln1(xs[2]), ln1(xblk(3))]
    for c in range(4):
        ats[0].q[c] = q_s[:, c * 128:(c + 1) * 128] + qhalf(1, c)
    qt(1, [0, 1, 2, 3])
    qt(2, [0, 1, 2, 3])
    wait(cp_wk)
    perm_qkv(1)
    qt(3, [0, 1])
    qt(0, [4, 5, 6, 7])
    qt(1, [4, 5, 6, 7])
    ats[0].qk_all()
    qt(3, [2, 3])
    qt(2, [4, 5, 6, 7])
    for c in range(NC):
        ats[1].qk(c)
    qt(3, [4, 5])
    ats[1].flush()
    wait(cp_wv, cp_wo, cp_b1, cp_b2)
    perm_qkv(2)
    wo_pieces = [functools.partial(fn, cb, t) for cb in range(4) for fn in (perm_wo_a, perm_wo_b) for t in range(4)]
    for k, fn in enumerate(wo_pieces):
        tl.trigger(tl.slot + 1 + k // 4, lambda piece, fn=fn: fn())
    for cb, s in enumerate(tl.rel((7, 9, 11, 13))):
        tl.deadline(s, lambda cb=cb: _or_all(wo_outs[cb]) & zero_s[...])
    l1 = lax.broadcasted_iota(jnp.int32, (1, 128), 1)
    b1_p[:, 1280:FP] = jnp.where(l1 == F - 1280, 4.0, 0.0)
    b1_p[:, 0:F] = b1_v[...].astype(f32).reshape(1, F) * 0.5
    rpad = lax.broadcasted_iota(jnp.int32, (FP - F, D), 0)
    w2_v[F:FP, :] = jnp.where(rpad == 0, b2_v[...].astype(f32).reshape(1, D) * 0.125, 0.0).astype(bf16)
    qt(3, [6, 7])
    qt(0, [8, 9, 10, 11])
    ats[0].due_at(tl.rel((3, 4, 4, 5, 6, 6, 7, 7)))
    qt(1, [8, 9, 10, 11])
    qt(2, [8, 9, 10, 11])
    halo(0, PB + P * M)
    ats[1].due_at(tl.rel((0, 1, 2, 3, 4, 5, 6, 7)))
    wblk(0)
    qt(3, [8, 9, 10, 11])
    y0 = ln2(xs[0])
    wait(cp_w1)
    ats[2].qk_all()
    ats[2].due_at(tl.rel((10, 12, 14, 16, 18, 20, 22, 24)))
    wblk(1)
    h0 = mm_M1(y0, repack=True)
    h1 = mm_M1(ln2(xs[1]))
    wblk(2)
    wait(cp_w2)
    x0 = mm_M2(xs[0], h0, repack=True)
    x1 = mm_M2(xs[1], h1)
    h2 = mm_M1(ln2(xs[2]))
    at0 = mm_Q(ln1(x0), 1, (5, 6, 7, 8, 9, 10, 11, 12), first=True, row0=PB)
    halo(1, PB + M)
    at1 = mm_Q(ln1(x1), 1, (10, 12, 14, 16, 18, 20, 22, 24))
    x0 = mm_W(x0, at0.done())
    x2 = mm_M2(xs[2], h2)
    h0 = mm_M1(ln2(x0))
    x1 = mm_W(x1, at1.done())
    halo(1, HALO + M)
    ats[3].start_at(tl.rel((0, 1, 2, 3, 4, 5, 6, 7)))
    put_out(0, mm_M2(x0, h0))
    ats[3].due_at(tl.rel(DL_LAST))
    h1 = mm_M1(ln2(x1))
    put_out(1, mm_M2(x1, h1))
    o3 = ats[3].done()
    halo(0, HALO + M)
    save(o3, x2)

    wait(cp_xr)

    def body(i, carry):
        o, x1 = load()
        for u in range(U):
            o, x1 = step(o, x1, P + i * U + u, last=(u == U - 1))
        save(o, x1)
        return carry
    lax.fori_loop(0, (NB - 1 - P) // U, body, 0)

    o, x1 = load()
    x1, x2 = step_a(o, x1, NB - 1)
    y2 = ln2(x2)
    at = mm_Q(ln1(x1), 1, DL_TAIL)
    h2 = mm_M1(y2)
    put_out(NB - 2, mm_M2(x2, h2, js=(0, 1)))
    x3 = mm_W(x1, at.done())
    put_out(NB - 2, mm_M2(x2, h2, js=(2, 3)), 256)
    h3 = mm_M1(ln2(x3))
    for j in range(4):
        put_out(NB - 1, mm_M2(x3, h3, js=(j,)), j * 128)
    cp(o_v, o_hbm, osem).wait()


@jax.jit
def pallas_interleave_layers__sliding_local_dilated__mixer_channel_mlp__prompt_kernel(
    A_x: jax.Array,
    A_wqkv: jax.Array,
    A_wo: jax.Array,
    B_x: jax.Array,
    B_w1: jax.Array,
    B_b1: jax.Array,
    B_w2: jax.Array,
    B_b2: jax.Array,
):
    assert (NB - 1 - P) % U == 0
    anyspec = pl.BlockSpec(memory_space=pl.ANY)
    out = pl.pallas_call(
        _kernel,
        in_specs=[anyspec] * 7,
        out_specs=anyspec,
        out_shape=jax.ShapeDtypeStruct((S, D), bf16),
        scratch_shapes=[
            pltpu.VMEM((S, D), bf16), pltpu.VMEM((S, D), bf16),
            pltpu.VMEM((D, 3 * D), bf16), pltpu.VMEM((D, D), bf16),
            pltpu.VMEM((F, D), bf16), pltpu.VMEM((FP, D), bf16),
            pltpu.VMEM((F,), bf16), pltpu.VMEM((D,), bf16),
            pltpu.VMEM((D // 2, 3 * D), u32), pltpu.VMEM((D // 2, D), u32),
            pltpu.VMEM((F // 2, D), u32), pltpu.VMEM((FP // 2, D), u32),
            pltpu.VMEM((1, FP), f32),
            pltpu.VMEM((4, H * WS, 128), f32),
            pltpu.VMEM((16, 4 * M + 2 * HALO, 128), f32),
            pltpu.VMEM((M // 2, D), u32), pltpu.VMEM((M, D), f32),
            pltpu.VMEM((M, D), f32),
            pltpu.VMEM((8, 128), u32),
            pltpu.SemaphoreType.DMA((12,)), pltpu.SemaphoreType.DMA(()),
        ],
        compiler_params=pltpu.CompilerParams(vmem_limit_bytes=100 << 20),
    )(A_x.reshape(S, D), A_wqkv, A_wo, B_w1.T, B_b1, B_w2, B_b2)
    return out.reshape(1, S, D)
```

```python
import functools
import math

import jax
import jax.numpy as jnp
import numpy as np
from jax import lax
import jax.experimental.pallas as pl
import jax.experimental.pallas.tpu as pltpu

S, D, F = 2048, 512, 1376
FP = 1408
H, DH, W, DIL = 32, 16, 8, 2
HALO = 16
WS = 20
WROWS = H * WS + 24
EPS = 1e-5
LOG2E = 1.4426950408889634
QSCALE = (DH ** -0.5) * LOG2E
QSCALE_BITS = int(np.float32(QSCALE).view(np.uint32))
NEG = -1e9 * LOG2E
f32, bf16, u32 = jnp.float32, jnp.bfloat16, jnp.uint32

M = 128
NB = S // M
RC = 16
RA = 16
NC = M // RA
P = 3
U = 2
PB = 2 * HALO + M

NB_SLOTS = (-5, -4, -3, -2, -1, 0, 1, 2)
DL_SLOTS = (15, 16, 17, 18, 19, 20, 21, 22)
DL_LAST = (14, 15, 16, 17, 18, 19, 20, 21)
DL_TAIL = (8, 9, 10, 12, 13, 14, 15, 16)
M1_ORDER = (0, 1, 2, 3, 10, 4, 5, 6, 7, 8, 9)


def _ln(x):
    m = jnp.mean(x, axis=-1, keepdims=True)
    xc = x - m
    v = jnp.mean(xc * xc, axis=-1, keepdims=True)
    return xc * lax.rsqrt(v + EPS)


def _ln_half(x):
    m = jnp.mean(x, axis=-1, keepdims=True)
    xc = x - m
    v4 = jnp.sum(xc * xc, axis=-1, keepdims=True) * (4.0 / D)
    return xc * lax.rsqrt(v4 + 4.0 * EPS)


def _gelu_from_half(z):
    c = math.sqrt(2.0 / math.pi)
    inner = z * (2.0 * c + (8.0 * c * 0.044715) * (z * z))
    return z + z * jnp.tanh(inner)


def _dot(a, b):
    return jnp.dot(a, b, preferred_element_type=f32)


def _dot_t(a, b):
    return lax.dot_general(a, b, (((1,), (1,)), ((), ())), preferred_element_type=f32)


def _or_all(xs):
    return functools.reduce(lambda u, v: u | v, xs)


def _pieces(a):
    return [a[r:r + 8, c:c + 128] for r in range(0, a.shape[0], 8) for c in range(0, a.shape[1], 128)]


def _patch(wu, r, tok):
    rows = wu[r:r + 8]
    if wu.shape[1] > 128:
        rows = jnp.concatenate([rows[:, 0:128] | tok, rows[:, 128:]], axis=1)
    else:
        rows = rows | tok
    parts = ([wu[:r]] if r > 0 else []) + [rows] + ([wu[r + 8:]] if r + 8 < wu.shape[0] else [])
    return jnp.concatenate(parts, axis=0)


class _Timeline:
    def __init__(self):
        self.slot, self.due, self.trig = 0, {}, {}

    def rel(self, offs):
        return [self.slot + o for o in offs]

    def deadline(self, slot, fn):
        self.due.setdefault(slot, []).append(fn)

    def trigger(self, slot, fn):
        self.trig.setdefault(slot, []).append(fn)

    def weights(self, wu, r=0, off=0):
        for fn in self.due.pop(self.slot + off, []):
            wu = _patch(wu, r, fn())
        return wu

    def done(self, r, n=1):
        lo = self.slot
        self.slot += n
        for s in range(lo, self.slot):
            for fn in self.trig.pop(s, []):
                fn(r[r.shape[0] - 8:, 0:128])

    def barrier(self):
        assert not self.trig
        self.due.clear()


def _kernel(x_hbm, wqkv_hbm, wo_hbm, w1t_hbm, b1_hbm, w2_hbm, b2_hbm, o_hbm,
            x_v, o_v, wqkv_v, wo_v, w1_v, w2_v, b1_v, b2_v,
            wqkv_p, wo_p, w1_p, w2_p, b1_p, wo_tmp, kv, o_s, q_s, x1_s, zero_s, sems):
    tl = _Timeline()

    XE = (P + 1) * M
    cp = pltpu.make_async_copy
    cp_x0 = cp(x_hbm.at[0:M], x_v.at[0:M], sems.at[0])
    cp_wq = [cp(wqkv_hbm.at[hf * 256:(hf + 1) * 256, 0:D], wqkv_v.at[hf * 256:(hf + 1) * 256, 0:D], sems.at[1 + hf])
             for hf in range(2)]
    cp_x123 = cp(x_hbm.at[M:XE], x_v.at[M:XE], sems.at[3])
    cp_wk = cp(wqkv_hbm.at[:, D:2 * D], wqkv_v.at[:, D:2 * D], sems.at[4])
    cp_wv = cp(wqkv_hbm.at[:, 2 * D:3 * D], wqkv_v.at[:, 2 * D:3 * D], sems.at[5])
    cp_wo = cp(wo_hbm, wo_v, sems.at[5])
    cp_b1 = cp(b1_hbm, b1_v, sems.at[5])
    cp_b2 = cp(b2_hbm, b2_v, sems.at[5])
    cp_w1 = cp(w1t_hbm, w1_v, sems.at[0])
    cp_w2 = cp(w2_hbm, w2_v.at[0:F], sems.at[1])
    cp_xr = cp(x_hbm.at[XE:S], x_v.at[XE:S], sems.at[2])
    osem = sems.at[3]
    for c_ in [cp_x0, cp_wq[0], cp_wq[1], cp_x123, cp_wk, cp_wv, cp_wo, cp_b1, cp_b2]:
        c_.start()

    def wait(*cps):
        tl.barrier()
        for c_ in cps:
            c_.wait()

    def rowslice(n):
        r = n * M
        if not isinstance(n, int):
            r = pl.multiple_of(r, M)
        return pl.ds(r, M)

    lane = lax.broadcasted_iota(jnp.int32, (8, 128), 1)
    dq = (lane % 16) // 4
    g_, j_, h_ = lane // 32, (lane % 32) // 8, lane % 8
    idx = [h_ * 16 + 4 * ((i + j_) % 4) + g_ for i in range(4)]
    msk = [dq == t for t in range(4)]

    def perm_qkv(t, rows=range(D // 16)):
        for i in range(4):
            for r in rows:
                src = [pltpu.bitcast(wqkv_v[r * 16:(r + 1) * 16, t * D + j * 128: t * D + (j + 1) * 128], u32)
                       for j in range(4)]
                m = src[(0 - i) % 4]
                for tq in range(1, 4):
                    m = jnp.where(msk[tq], src[(tq - i) % 4], m)
                wqkv_p[r * 8:(r + 1) * 8, t * D + i * 128: t * D + (i + 1) * 128] = \
                    jnp.take_along_axis(m, idx[i], axis=1)

    wo_outs = [[] for _ in range(4)]

    def perm_wo_a(cb, j):
        for hh in range(8 * j, 8 * j + 8):
            wo_tmp[cb, hh * WS:hh * WS + DH, :] = wo_v[hh * DH:(hh + 1) * DH, cb * 128:(cb + 1) * 128].astype(f32)

    def perm_wo_b(cb, i):
        for g in range(4):
            rows = [wo_tmp[cb, pl.ds(j * 8 * WS + 4 * ((i + j) % 4) + g, 8, stride=WS), :] for j in range(4)]
            blk = pltpu.bitcast(jnp.concatenate(rows, axis=0).astype(bf16), u32)
            r0 = (i * 128 + g * 32) // 2
            wo_p[r0:r0 + 16, cb * 128:(cb + 1) * 128] = blk
            wo_outs[cb] += [blk[0:8], blk[8:16]]

    def ztok(pieces):
        return _or_all([pltpu.bitcast(p, u32) for p in pieces]) & zero_s[...]

    def rows_map(fn, x):
        return jnp.concatenate([fn(x[r:r + RC]) for r in range(0, x.shape[0], RC)], axis=0)

    def ln1(x):
        return rows_map(_ln, x).astype(bf16)

    def ln2(x):
        return rows_map(lambda a: _ln_half(_ln(a)), x).astype(bf16)

    def halo(layer, end):
        L = layer * 8
        kv[L:L + 8, 0:HALO, :] = kv[L:L + 8, end - HALO:end, :]

    class Attn:
        def __init__(self, layer, first=False, row0=HALO):
            self.layer, self.first, self.row0 = layer, first, row0
            self.q = [None] * 4
            self.half, self.logit, self.outs = {}, {}, {}

        def qk(self, c, tok=None):
            L, r0 = self.layer * 8, c * RA
            g0 = self.row0 + r0
            if tok is None:
                sc = QSCALE
            else:
                sc = jnp.concatenate([pltpu.bitcast(tok | QSCALE_BITS, f32)] * (RA // 8), axis=0)
            qs = [self.q[j][r0:r0 + RA] * sc for j in range(4)]
            ls = []
            for w in range(W):
                s = None
                for j in range(4):
                    t = qs[j] * kv[L + j, pl.ds(g0 - DIL * w, RA), :]
                    s = t if s is None else s + t
                ls.append(s)
            self.half[c] = [s + pltpu.roll(s, 64, 1) for s in ls]
            for c2 in sorted(self.half):
                if c2 < c:
                    self.qkb(c2)

        def qkb(self, c):
            r0 = c * RA
            ls = [s + pltpu.roll(s, 32, 1) for s in self.half.pop(c)]
            if self.first and r0 < HALO:
                row = r0 + lax.broadcasted_iota(jnp.int32, (RA, 128), 0)
                ls = [ls[0]] + [jnp.where(row >= DIL * w, ls[w], NEG) for w in range(1, W)]
            self.logit[c] = ls

        def flush(self):
            for c in sorted(self.half):
                self.qkb(c)

        def qk_all(self):
            for c in range(NC):
                self.qk(c)
            self.flush()

        def av(self, c):
            L, r0 = self.layer * 8, c * RA
            g0 = self.row0 + r0
            ls = self.logit[c]
            m = ls[0]
            for w in range(1, W):
                m = jnp.maximum(m, ls[w])
            ps = [jnp.exp2(l - m) for l in ls]
            den = ps[0]
            for w in range(1, W):
                den = den + ps[w]
            inv = pl.reciprocal(den, approx=True)
            inv = inv * (2.0 - den * inv)
            oj = []
            for j in range(4):
                a = None
                for w in range(W):
                    t = ps[w] * kv[L + 4 + j, pl.ds(g0 - DIL * w, RA), :]
                    a = t if a is None else a + t
                oj.append(a * inv)
            self.outs[c] = jnp.concatenate(oj, axis=1)

        def finish(self, c):
            assert c in self.logit or c in self.half
            if c in self.half:
                self.qkb(c)
            if c not in self.outs:
                self.av(c)

        def start_at(self, slots):
            for c, s in enumerate(slots):
                tl.trigger(s, lambda piece, c=c: self.qk(c, ztok([piece])))

        def due_at(self, slots):
            def tok(c):
                self.finish(c)
                return ztok(_pieces(self.outs[c]))
            for c, s in enumerate(slots):
                tl.deadline(s, lambda c=c: tok(c))

        def done(self):
            for c in range(NC):
                self.finish(c)
            return jnp.concatenate([self.outs[c] for c in range(NC)], axis=0).astype(bf16)

    def q_tile(at, y, c):
        wu = tl.weights(wqkv_p[:, c * 128:(c + 1) * 128])
        r = _dot(y, pltpu.bitcast(wu, bf16))
        if c < 4:
            at.q[c] = r
        else:
            kv[at.layer * 8 + c - 4, at.row0:at.row0 + M, :] = r
        tl.done(r)

    def mm_Q(y, layer, dl, first=False, row0=HALO):
        at = Attn(layer, first=first, row0=row0)
        end = tl.slot + 12
        at.start_at([end + s for s in NB_SLOTS])
        at.due_at([end + s for s in dl])
        for c in range(12):
            q_tile(at, y, c)
        return at

    def mm_W(x, o):
        outs = []
        for j in range(4):
            cs = slice(j * 128, (j + 1) * 128)
            r = _dot(o, pltpu.bitcast(tl.weights(wo_p[:, cs]), bf16))
            tl.done(r)
            outs.append(x[:, cs] + r)
        return jnp.concatenate(outs, axis=1)

    def mm_M1(y, repack=False):
        hs = {}
        for t in M1_ORDER:
            n0 = t * 128
            nr = min(128, F - n0)
            if repack:
                wu = pltpu.bitcast(w1_v[n0:n0 + nr, :], u32)
                w1_p[n0 // 2:(n0 + nr) // 2, :] = wu
            else:
                wu = w1_p[n0 // 2:(n0 + nr) // 2, :]
            w = pltpu.bitcast(tl.weights(wu), bf16)
            if nr == 128:
                r = _dot_t(y, w)
                tl.done(r)
            else:
                rt = _dot_t(w, y)
                tl.done(rt)
                r = jnp.concatenate([rt, jnp.zeros((128 - nr, M), f32)], axis=0).T
            hs[t] = _gelu_from_half(r + b1_p[:, n0:n0 + 128])
        return jnp.concatenate([hs[t] for t in range(FP // 128)], axis=1).astype(bf16)

    def mm_M2(x, h, repack=False, js=(0, 1, 2, 3)):
        outs = []
        for j in js:
            cs = slice(j * 128, (j + 1) * 128)
            if repack:
                wu = pltpu.bitcast(w2_v[:, cs], u32)
                w2_p[:, cs] = wu
            else:
                wu = w2_p[:, cs]
            ps = [p for p in range(11) if (4 * p) // 11 == j]
            for i, p in enumerate(ps):
                wu = tl.weights(wu, ((4 * p) % 11) * 64, off=i)
            r = _dot(h, pltpu.bitcast(wu, bf16))
            tl.done(r, len(ps))
            outs.append(x[:, cs] + r)
        return jnp.concatenate(outs, axis=1)

    def xblk(n):
        return x_v[rowslice(n), :].astype(f32)

    def put_out(n, val, c0=0):
        cs = slice(c0, c0 + val.shape[1])
        o_v[rowslice(n), cs] = val.astype(bf16)
        cp(o_v.at[rowslice(n), cs], o_hbm.at[rowslice(n), cs], osem).start()

    def save(o, x1):
        x1_s[...] = x1
        o_s[...] = pltpu.bitcast(o, u32)
        tl.barrier()

    def load():
        return pltpu.bitcast(o_s[...], bf16), x1_s[...]

    def step_a(o, x1, n):
        x = mm_W(xblk(n), o)
        y = ln2(x)
        at = mm_Q(ln1(x1), 1, DL_SLOTS)
        h = mm_M1(y)
        x1n = mm_M2(x, h)
        x2 = mm_W(x1, at.done())
        halo(1, HALO + M)
        return x1n, x2

    def step(o, x1, n, last):
        x1n, x2 = step_a(o, x1, n)
        y2 = ln2(x2)
        at = mm_Q(ln1(xblk(n + 1)), 0, DL_LAST if last else DL_SLOTS)
        h2 = mm_M1(y2)
        put_out(n - 1, mm_M2(x2, h2))
        on = at.done()
        halo(0, HALO + M)
        return on, x1n

    kv[:, PB - HALO:PB, :] = jnp.zeros((16, HALO, 128), f32)
    zero_s[...] = jnp.zeros((8, 128), u32)
    wo_tmp[...] = jnp.zeros((4, WROWS, 128), f32)
    ats = [Attn(0, first=(b == 0), row0=PB + b * M) for b in range(P)] + [Attn(0)]

    def qt(b, cs):
        for c in cs:
            q_tile(ats[b], ys[b], c)

    def wblk(b):
        xs[b] = mm_W(xs[b], ats[b].done())

    def qhalf(hf, c):
        w = pltpu.bitcast(wqkv_p[hf * 128:(hf + 1) * 128, c * 128:(c + 1) * 128], bf16)
        return _dot(ys[0][:, hf * 256:(hf + 1) * 256], w)

    wait(cp_x0)
    cp_w1.start()
    xs = [xblk(0)]
    ys = [ln1(xs[0])]
    wait(cp_wq[0])
    cp_w2.start()
    perm_qkv(0, rows=range(0, 16))
    for c in range(4):
        q_s[:, c * 128:(c + 1) * 128] = qhalf(0, c)
    wait(cp_wq[1])
    cp_xr.start()
    perm_qkv(0, rows=range(16, 32))
    wait(cp_x123)
    xs += [xblk(1), xblk(2)]
    ys += [ln1(xs[1]), ln1(xs[2]), ln1(xblk(3))]
    for c in range(4):
        ats[0].q[c] = q_s[:, c * 128:(c + 1) * 128] + qhalf(1, c)
    qt(1, [0, 1, 2, 3])
    qt(2, [0, 1, 2, 3])
    wait(cp_wk)
    perm_qkv(1)
    qt(3, [0, 1])
    qt(0, [4, 5, 6, 7])
    qt(1, [4, 5, 6, 7])
    ats[0].qk_all()
    qt(3, [2, 3])
    qt(2, [4, 5, 6, 7])
    for c in range(NC):
        ats[1].qk(c)
    qt(3, [4, 5])
    ats[1].flush()
    wait(cp_wv, cp_wo, cp_b1, cp_b2)
    perm_qkv(2)
    wo_pieces = [functools.partial(fn, cb, t) for cb in range(4) for fn in (perm_wo_a, perm_wo_b) for t in range(4)]
    for k, fn in enumerate(wo_pieces):
        tl.trigger(tl.slot + 1 + k // 4, lambda piece, fn=fn: fn())
    for cb, s in enumerate(tl.rel((7, 9, 11, 13))):
        tl.deadline(s, lambda cb=cb: _or_all(wo_outs[cb]) & zero_s[...])
    l1 = lax.broadcasted_iota(jnp.int32, (1, 128), 1)
    b1_p[:, 1280:FP] = jnp.where(l1 == F - 1280, 4.0, 0.0)
    b1_p[:, 0:F] = b1_v[...].astype(f32).reshape(1, F) * 0.5
    rpad = lax.broadcasted_iota(jnp.int32, (FP - F, D), 0)
    w2_v[F:FP, :] = jnp.where(rpad == 0, b2_v[...].astype(f32).reshape(1, D) * 0.125, 0.0).astype(bf16)
    qt(3, [6, 7])
    qt(0, [8, 9, 10, 11])
    ats[0].due_at(tl.rel((3, 4, 4, 5, 6, 6, 7, 7)))
    qt(1, [8, 9, 10, 11])
    qt(2, [8, 9, 10, 11])
    halo(0, PB + P * M)
    ats[1].due_at(tl.rel((0, 1, 2, 3, 4, 5, 6, 7)))
    wblk(0)
    qt(3, [8, 9, 10, 11])
    y0 = ln2(xs[0])
    wait(cp_w1)
    ats[2].qk_all()
    ats[2].due_at(tl.rel((10, 12, 14, 16, 18, 20, 22, 24)))
    wblk(1)
    h0 = mm_M1(y0, repack=True)
    h1 = mm_M1(ln2(xs[1]))
    wblk(2)
    wait(cp_w2)
    x0 = mm_M2(xs[0], h0, repack=True)
    x1 = mm_M2(xs[1], h1)
    h2 = mm_M1(ln2(xs[2]))
    at0 = mm_Q(ln1(x0), 1, (5, 6, 7, 8, 9, 10, 11, 12), first=True, row0=PB)
    halo(1, PB + M)
    at1 = mm_Q(ln1(x1), 1, (10, 12, 14, 16, 18, 20, 22, 24))
    x0 = mm_W(x0, at0.done())
    x2 = mm_M2(xs[2], h2)
    h0 = mm_M1(ln2(x0))
    x1 = mm_W(x1, at1.done())
    halo(1, HALO + M)
    ats[3].start_at(tl.rel((0, 1, 2, 3, 4, 5, 6, 7)))
    put_out(0, mm_M2(x0, h0))
    ats[3].due_at(tl.rel(DL_LAST))
    h1 = mm_M1(ln2(x1))
    put_out(1, mm_M2(x1, h1))
    o3 = ats[3].done()
    halo(0, HALO + M)
    save(o3, x2)

    wait(cp_xr)

    def body(i, carry):
        o, x1 = load()
        for u in range(U):
            o, x1 = step(o, x1, P + i * U + u, last=(u == U - 1))
        save(o, x1)
        return carry
    lax.fori_loop(0, (NB - 1 - P) // U, body, 0)

    o, x1 = load()
    x1, x2 = step_a(o, x1, NB - 1)
    y2 = ln2(x2)
    at = mm_Q(ln1(x1), 1, DL_TAIL)
    h2 = mm_M1(y2)
    put_out(NB - 2, mm_M2(x2, h2, js=(0, 1)))
    x3 = mm_W(x1, at.done())
    put_out(NB - 2, mm_M2(x2, h2, js=(2, 3)), 256)
    h3 = mm_M1(ln2(x3))
    for j in range(4):
        put_out(NB - 1, mm_M2(x3, h3, js=(j,)), j * 128)
    cp(o_v, o_hbm, osem).wait()


@jax.jit
def pallas_interleave_layers__sliding_local_dilated__mixer_channel_mlp__prompt_kernel(
    A_x: jax.Array,
    A_wqkv: jax.Array,
    A_wo: jax.Array,
    B_x: jax.Array,
    B_w1: jax.Array,
    B_b1: jax.Array,
    B_w2: jax.Array,
    B_b2: jax.Array,
):
    assert (NB - 1 - P) % U == 0
    anyspec = pl.BlockSpec(memory_space=pl.ANY)
    out = pl.pallas_call(
        _kernel,
        in_specs=[anyspec] * 7,
        out_specs=anyspec,
        out_shape=jax.ShapeDtypeStruct((S, D), bf16),
        scratch_shapes=[
            pltpu.VMEM((S, D), bf16), pltpu.VMEM((S, D), bf16),
            pltpu.VMEM((D, 3 * D), bf16), pltpu.VMEM((D, D), bf16),
            pltpu.VMEM((F, D), bf16), pltpu.VMEM((FP, D), bf16),
            pltpu.VMEM((F,), bf16), pltpu.VMEM((D,), bf16),
            pltpu.VMEM((D // 2, 3 * D), u32), pltpu.VMEM((D // 2, D), u32),
            pltpu.VMEM((F // 2, D), u32), pltpu.VMEM((FP // 2, D), u32),
            pltpu.VMEM((1, FP), f32),
            pltpu.VMEM((4, WROWS, 128), f32),
            pltpu.VMEM((16, 4 * M + 2 * HALO, 128), f32),
            pltpu.VMEM((M // 2, D), u32), pltpu.VMEM((M, D), f32),
            pltpu.VMEM((M, D), f32),
            pltpu.VMEM((8, 128), u32),
            pltpu.SemaphoreType.DMA((6,)),
        ],
        compiler_params=pltpu.CompilerParams(vmem_limit_bytes=100 << 20),
    )(A_x.reshape(S, D), A_wqkv, A_wo, B_w1.T, B_b1, B_w2, B_b2)
    return out.reshape(1, S, D)
```
